```python
import jax
import jax.numpy as jnp

def _softmax(x, axis=-1):
    return jax.nn.softmax(x, axis=axis)
def _gelu(x):
    return jax.nn.gelu(x, approximate=True)
def _silu(x):
    return jax.nn.silu(x)
def _sigmoid(x):
    return jax.nn.sigmoid(x)
def _layernorm(x, axis=-1, eps=1e-5):
    m = jnp.mean(x, axis=axis, keepdims=True)
    v = jnp.var(x, axis=axis, keepdims=True)
    return (x - m) / jnp.sqrt(v + eps)
def _scatter_add(tgt, idx, src, axis=0):
    return tgt.at[idx].add(src)
def _segment_sum(src, seg, n):
    return jax.ops.segment_sum(src, seg, n)
class _Rng:
    def __init__(self, key):
        self._k = key
    def _next(self):
        self._k, sub = jax.random.split(self._k)
        return sub
    def normal(self, shape):
        return jax.random.normal(self._next(), shape, dtype=jnp.bfloat16)
    def randint(self, lo, hi, shape):
        return jax.random.randint(self._next(), shape, lo, hi, dtype=jnp.int32)
    def uniform(self, shape, lo=0.0, hi=1.0):
        return jax.random.uniform(self._next(), shape, jnp.bfloat16, lo, hi)
    def permutation(self, n):
        return jax.random.permutation(self._next(), n)


kernel_name = 'interleave_layers__linear_attn_block__mixer_channel_mlp__prompt'

def _fwd_setup_inputs():
    _rng = _Rng(jax.random.key(int.from_bytes(__import__("os").urandom(4), "little")))
    _w = (lambda a: (lambda t: t.astype(jnp.bfloat16) if jnp.issubdtype(t.dtype, jnp.floating) else t)(jnp.asarray(a)))
    def _A_setup():
        B, S, D = 1, 2048, 576
        return {
            "x": _w((lambda *s: _rng.normal(s) * 0.05)(B, S, D)),
            "wqkv": _w((lambda *s: _rng.normal(s) * 0.05)(D, 3 * D)),
            "wo": _w((lambda *s: _rng.normal(s) * 0.05)(D, D)),
        }
    _A_in = _A_setup()

    def _B_setup():
        B, S, D, F = 1, 2048, 576, 4608
        return {
            "x": _w((lambda *s: _rng.normal(s) * 0.05)(B, S, D)),
            "w1": _w((lambda *s: _rng.normal(s) * 0.05)(D, F) * (D ** -0.5)),
            "b1": _w((lambda *s: _rng.normal(s) * 0.05)(F)),
            "w2": _w((lambda *s: _rng.normal(s) * 0.05)(F, D) * (F ** -0.5)),
            "b2": _w((lambda *s: _rng.normal(s) * 0.05)(D)),
        }
    _B_in = _B_setup()

    return {
        "A_x": _A_in["x"],
        "A_wqkv": _A_in["wqkv"],
        "A_wo": _A_in["wo"],
        "B_x": _B_in["x"],
        "B_w1": _B_in["w1"],
        "B_b1": _B_in["b1"],
        "B_w2": _B_in["w2"],
        "B_b2": _B_in["b2"],
    }

def _fwd_reference(A_x, A_wqkv, A_wo, B_x, B_w1, B_b1, B_w2, B_b2):
    def _A_ref(x, wqkv, wo):
        B, S, D = x.shape
        H = 32; Dh = D // H
        qkv = (lambda x, *d: x.transpose(*d))((x @ wqkv).reshape(B, S, 3, H, Dh), 2, 0, 3, 1, 4)
        q, k, v = qkv[0], qkv[1], qkv[2]
        phi = lambda t: jnp.where(t > 0, t + 1, jnp.exp(t)) + 1e-6
        pq, pk = phi(q), phi(k)
        kv = jnp.einsum("bhsd,bhse->bhde", pk, v)
        z = jnp.einsum("bhsd->bhd", pk)
        num = jnp.einsum("bhqd,bhde->bhqe", pq, kv)
        den = jnp.einsum("bhqd,bhd->bhq", pq, z)[..., None] + 1e-6
        o = num / den
        return (lambda x, *d: x.transpose(*d))(o, 0, 2, 1, 3).reshape(B, S, D) @ wo

    def _B_ref(x, w1, b1, w2, b2):
        y = _layernorm(x, axis=-1)
        h = _gelu(jnp.einsum("bsd,df->bsf", y, w1) + b1)
        return jnp.einsum("bsf,fd->bsd", h, w2) + b2

    x = A_x
    x = x + _A_ref(_layernorm(x, axis=-1), A_wqkv, A_wo)
    x = x + _B_ref(_layernorm(x, axis=-1), B_w1, B_b1, B_w2, B_b2)
    x = x + _A_ref(_layernorm(x, axis=-1), A_wqkv, A_wo)
    x = x + _B_ref(_layernorm(x, axis=-1), B_w1, B_b1, B_w2, B_b2)
    return x


def setup_inputs():
    _inp = _fwd_setup_inputs()
    _gk = jax.random.fold_in(jax.random.key(int.from_bytes(__import__("os").urandom(4), "little")), 2**31 - 1)
    _shapes = [[1, 2048, 576]]
    _dtypes = ['bfloat16']
    _gks = jax.random.split(_gk, len(_shapes))
    _gs = [jax.random.normal(k, s, dtype=jnp.dtype(d)) * 0.05 for k, s, d in zip(_gks, _shapes, _dtypes)]
    _inp["grad_out"] = _gs[0]
    return _inp

def reference(A_x, A_wqkv, A_wo, B_w1, B_b1, B_w2, B_b2, B_x, grad_out):
    _const = dict(B_x=B_x)
    def _f(*_d):
        return _fwd_reference(**{'A_x': _d[0], 'A_wqkv': _d[1], 'A_wo': _d[2], 'B_w1': _d[3], 'B_b1': _d[4], 'B_w2': _d[5], 'B_b2': _d[6], **_const})
    _out, _vjp = jax.vjp(_f, A_x, A_wqkv, A_wo, B_w1, B_b1, B_w2, B_b2)
    _grads = _vjp(grad_out)
    _out0 = jnp.asarray(_out)
    return (_out0, *[jnp.asarray(_g) for _g in _grads])
```

```python
import functools

import jax
import jax.numpy as jnp
from jax import lax
import jax.experimental.pallas as pl
import jax.experimental.pallas.tpu as pltpu

S, D, F, H, DH = 2048, 576, 4608, 32, 18
EPS = 1e-5
PEPS = 1e-6
BF = jnp.bfloat16
F32 = jnp.float32
NN = (((1,), (0,)), ((), ()))
NT = (((1,), (1,)), ((), ()))
C0 = 0.7978845608028654
C1 = 0.7978845608028654 * 0.044715

PIECES = ((0, 144, 0, 128), (112, 272, 128, 256), (240, 400, 256, 384), (368, 528, 384, 512),
          (496, 576, 512, 576))

TS = 512
TF1 = 512
TF2 = 256
TF3 = 256
NTS = S // TS


def _dot(a, b, dn=NN):
    return lax.dot_general(a, b, dn, preferred_element_type=F32)


def _assemble(ps):
    segs = []
    for j, (r0, r1, _, _) in enumerate(PIECES):
        lo = r0 if j == 0 else PIECES[j - 1][1]
        hi = r1 if j == len(PIECES) - 1 else PIECES[j + 1][0]
        segs.append(ps[j][lo - r0:hi - r0])
        if j != len(PIECES) - 1:
            segs.append(ps[j][hi - r0:r1 - r0] + ps[j + 1][0:r1 - hi])
    return jnp.concatenate(segs, axis=0)


def _bd_left(bd_ref, rhs_rows):
    return _assemble([_dot(bd_ref[r0:r1, t0:t1], rhs_rows(t0, t1)) for (r0, r1, t0, t1) in PIECES])


def _lanesum(a):
    acc = a[:, 0:128]
    for i in range(1, a.shape[1] // 128):
        acc = acc + a[:, i * 128:(i + 1) * 128]
    return acc


def _tile_lanes(col128, n):
    return col128 if n == 128 else jnp.concatenate([col128] * (n // 128), axis=1)


def _colmean(a):
    return jnp.sum(a, axis=0, keepdims=True) * (1.0 / D)


def _gelu_parts(pre, with_grad):
    u = pre * pre
    t = jnp.tanh(pre * (C0 + C1 * u))
    hp = 0.5 * pre
    h = hp + hp * t
    if not with_grad:
        return h, None
    gp = 0.5 + 0.5 * t + hp * (1.0 - t * t) * (C0 + (3.0 * C1) * u)
    return h, gp


def _kernel(x_hbm, g_hbm, wqkv_hbm, wo_hbm, w1_hbm, b1_hbm, w2_hbm, b2_hbm,
            out_hbm, dx_hbm, dwqkv_hbm, dwo_hbm, dw1_hbm, db1_hbm, dw2_hbm, db2_hbm,
            xin, gin, wqkv, wo, w1, w2, b1, b2,
            X, DY, N0, N1, Y0, Y1, QK0, QK1, PRE, YN, GN, STAT,
            wqkT, wv, wvT, wcat, bmask, b2c,
            G0, G1, KV0, KV1, KVT0, KVT1, M0, M1, MT, ZM, ZC0, ZC1,
            ACC, ZACC, DG, DKV, DKVT, DZC,
            DW1, DW2, DB1, DB2, DWQK, DWVT, DWO, db1s, db2s,
            sem_in, sem_x, sem_out, sem_o, sem_dx, sem_w1, sem_w2):
    Ns, Ys, QKs = (N0, N1), (Y0, Y1), (QK0, QK1)
    Gs, KVs, KVTs, Ms, ZCs = (G0, G1), (KV0, KV1), (KVT0, KVT1), (M0, M1), (ZC0, ZC1)

    def cols(t):
        return pl.ds(pl.multiple_of(t * TS, TS), TS)

    def x_copy(t):
        return pltpu.make_async_copy(x_hbm.at[:, cols(t)], xin.at[:, cols(t)], sem_x.at[t])

    in_copies = [
        pltpu.make_async_copy(wqkv_hbm, wqkv, sem_in.at[0]),
        pltpu.make_async_copy(wo_hbm, wo, sem_in.at[1]),
        pltpu.make_async_copy(b2_hbm, b2, sem_in.at[2]),
        pltpu.make_async_copy(b1_hbm, b1, sem_in.at[3]),
        pltpu.make_async_copy(w1_hbm, w1, sem_in.at[4]),
        pltpu.make_async_copy(w2_hbm, w2, sem_in.at[5]),
        pltpu.make_async_copy(g_hbm, gin, sem_in.at[6]),
    ]
    in_copies[0].start()
    for t in range(NTS):
        x_copy(t).start()
    for c in in_copies[1:]:
        c.start()

    ri = lax.broadcasted_iota(jnp.int32, (D, D), 0).astype(F32)
    ci = lax.broadcasted_iota(jnp.int32, (D, D), 1).astype(F32)
    same = jnp.floor((ri + 0.5) * (1.0 / DH)) == jnp.floor((ci + 0.5) * (1.0 / DH))
    bmask[...] = jnp.where(same, 1.0, 0.0).astype(BF)
    DWQK[...] = jnp.zeros(DWQK.shape, F32)
    DWVT[...] = jnp.zeros(DWVT.shape, F32)
    DWO[...] = jnp.zeros(DWO.shape, F32)
    DB2[...] = jnp.zeros(DB2.shape, F32)

    in_copies[0].wait()
    wqkT[...] = wqkv[:, 0:2 * D].astype(F32).T.astype(BF)
    wvv = wqkv[:, 2 * D:3 * D]
    wv[...] = wvv
    wvT[...] = wvv.astype(F32).T.astype(BF)
    wcat[:, 0:2 * D] = wqkv[:, 0:2 * D]

    def phase_c(l):
        ACC[...] = jnp.zeros(ACC.shape, F32)
        ZACC[...] = jnp.zeros(ZACC.shape, F32)

        def body(t, carry):
            cs = cols(t)
            if l == 0:
                x_copy(t).wait()
                x = xin[:, cs].astype(F32)
                X[:, cs] = x
            else:
                x = X[:, cs]
            c = x - _colmean(x)
            r = lax.rsqrt(_colmean(c * c) + EPS)
            n = (c * r).astype(BF)
            Ns[l][:, cs] = n
            STAT[l:l + 1, cs] = r
            qk = _dot(wqkT[...], n)
            ph = jnp.where(qk > 0, qk + 1.0, jnp.exp(jnp.minimum(qk, 0.0))) + PEPS
            QKs[l][0:D, cs] = ph[0:D].astype(BF)
            pk = ph[D:2 * D]
            pkb = pk.astype(BF)
            QKs[l][2 * D:3 * D, cs] = pkb
            ACC[...] += _dot(pkb, n, NT)
            ZACC[...] += _lanesum(pk)
            return carry

        lax.fori_loop(0, NTS, body, 0)

    def fin_fwd(l):
        Gs[l][...] = ACC[...].astype(BF)
        KVs[l][...] = jnp.zeros((D, D), BF)
        KVTs[l][...] = jnp.zeros((D, D), BF)
        for (r0, r1, t0, t1) in PIECES:
            mk = bmask[r0:r1, t0:t1].astype(F32)
            KVs[l][r0:r1, t0:t1] = (_dot(Gs[l][r0:r1, :], wv[:, t0:t1]) * mk).astype(BF)
            KVTs[l][r0:r1, t0:t1] = (_dot(wvT[r0:r1, :], Gs[l][t0:t1, :], NT) * mk).astype(BF)
        m = _bd_left(KVs[l], lambda t0, t1: wo[t0:t1, :])
        Ms[l][...] = m.astype(BF)
        MT[...] = m.T.astype(BF)
        za = ZACC[...]
        zrow = jnp.sum(za.T, axis=0, keepdims=True)
        ZM[...] = (bmask[...].astype(F32) * zrow).astype(BF)
        ZCs[l][...] = jnp.broadcast_to(jnp.sum(za, axis=1, keepdims=True), (D, 128))

    def phase_a(l):
        def body(t, carry):
            cs = cols(t)
            den = _bd_left(ZM, lambda t0, t1: QKs[l][t0:t1, cs]) + PEPS
            rden = 1.0 / den
            pq = QKs[l][0:D, cs].astype(F32)
            p = (pq * rden).astype(BF)
            QKs[l][D:2 * D, cs] = p
            QKs[l][0:D, cs] = (rden * jnp.minimum(pq - PEPS, 1.0)).astype(BF)
            x = X[:, cs] + _dot(MT[...], p)
            c = x - _colmean(x)
            s = lax.rsqrt((1.0 + EPS) * _colmean(c * c) + EPS * EPS)
            y = c * s
            Ys[l][:, cs] = y.astype(BF)
            STAT[2 + l:3 + l, cs] = s
            YN[cs, :] = y.T.astype(BF)
            X[:, cs] = x + _tile_lanes(b2c[...], TS)
            if l == 1:
                g = gin[:, cs].astype(F32)
                GN[cs, :] = g.T.astype(BF)
                DB2[...] += _lanesum(g)
                DY[:, cs] = jnp.zeros((D, TS), F32)
            return carry

        lax.fori_loop(0, NTS, body, 0)

    def mlp_fwd():
        def body(j, carry):
            fc = pl.ds(pl.multiple_of(j * TF1, TF1), TF1)
            pre = _dot(YN[...], w1[:, fc]) + b1[:, fc].astype(F32)
            PRE[:, fc] = pre.astype(BF)
            h, _ = _gelu_parts(pre, False)
            X[...] += _dot(w2[:, fc], h.astype(BF), NT)
            return carry

        lax.fori_loop(0, F // TF1, body, 0)

    def mlp_fwd_bwd():
        def body(j, carry):
            fc = pl.ds(pl.multiple_of(j * TF2, TF2), TF2)
            w1c = w1[:, fc]
            w2c = w2[:, fc]
            pre = _dot(YN[...], w1c) + b1[:, fc].astype(F32)
            dh = _dot(GN[...], w2c)
            h, gp = _gelu_parts(pre, True)
            hb = h.astype(BF)
            dpre = dh * gp
            dpb = dpre.astype(BF)
            DB1[:, fc] = jnp.sum(dpre.reshape(S // 8, 8, TF2), axis=0)
            X[...] += _dot(w2c, hb, NT)
            DW2[:, fc] = _dot(gin[...], hb)
            DY[...] += _dot(w1c, dpb, NT)
            DW1[:, fc] = _dot(Y1[...], dpb)
            return carry

        lax.fori_loop(0, F // TF2, body, 0)

    def w_out_copies(j):
        fc = pl.ds(pl.multiple_of(j * TF3, TF3), TF3)
        return (pltpu.make_async_copy(w1.at[:, fc], dw1_hbm.at[:, fc], sem_w1.at[j]),
                pltpu.make_async_copy(w2.at[:, fc], dw2_hbm.at[:, fc], sem_w2.at[j]))

    def mlp_bwd():
        def body(j, carry):
            fc = pl.ds(pl.multiple_of(j * TF3, TF3), TF3)
            w1c = w1[:, fc]
            w2c = w2[:, fc]
            pre = PRE[:, fc].astype(F32)
            dh = _dot(GN[...], w2c)
            h, gp = _gelu_parts(pre, True)
            hb = h.astype(BF)
            dpre = dh * gp
            dpb = dpre.astype(BF)
            DB1[:, fc] += jnp.sum(dpre.reshape(S // 8, 8, TF3), axis=0)
            DY[...] += _dot(w1c, dpb, NT)
            w2[:, fc] = (DW2[:, fc] + _dot(Y1[...], hb)).astype(BF)
            w1[:, fc] = (DW1[:, fc] + _dot(Y0[...], dpb)).astype(BF)
            for c in w_out_copies(j):
                c.start()
            return carry

        lax.fori_loop(0, F // TF3, body, 0)

    def out_copy(t):
        return pltpu.make_async_copy(gin.at[:, cols(t)], out_hbm.at[:, cols(t)], sem_o.at[t])

    def dx_copy(t):
        return pltpu.make_async_copy(xin.at[:, cols(t)], dx_hbm.at[:, cols(t)], sem_dx.at[t])

    def phase_e(l):
        ACC[...] = jnp.zeros(ACC.shape, F32)
        ZACC[...] = jnp.zeros(ZACC.shape, F32)

        def body(t, carry):
            cs = cols(t)
            if l == 1:
                g = gin[:, cs].astype(F32)
                gin[:, cs] = X[:, cs].astype(BF)
                out_copy(t).start()
            else:
                g = X[:, cs]
            y = Ys[l][:, cs].astype(F32)
            dy = DY[:, cs]
            s = STAT[2 + l:3 + l, cs]
            dx = g + s * (dy - _colmean(dy) - y * ((1.0 + EPS) * _colmean(dy * y)))
            X[:, cs] = dx
            dxb = dx.astype(BF)
            dp = _dot(Ms[l][...], dxb)
            pb = QKs[l][D:2 * D, cs]
            ACC[...] += _dot(pb, dxb, NT)
            p = pb.astype(F32)
            tt = (dp * p).astype(BF)
            hs = _bd_left(bmask, lambda t0, t1: tt[t0:t1])
            cq = QKs[l][0:D, cs].astype(F32)
            QKs[l][0:D, cs] = (cq * (dp - _tile_lanes(ZCs[l][...], TS) * hs)).astype(BF)
            ZACC[...] += _lanesum(p * hs)
            return carry

        lax.fori_loop(0, NTS, body, 0)

    def fin_bwd(l):
        DG[...] = ACC[...].astype(BF)
        DKV[...] = jnp.zeros((D, D), BF)
        DKVT[...] = jnp.zeros((D, D), BF)
        for (r0, r1, t0, t1) in PIECES:
            mk = bmask[r0:r1, t0:t1].astype(F32)
            DKV[r0:r1, t0:t1] = (_dot(DG[r0:r1, :], wo[t0:t1, :], NT) * mk).astype(BF)
            DKVT[r0:r1, t0:t1] = (_dot(wo[r0:r1, :], DG[t0:t1, :], NT) * mk).astype(BF)
        DWO[...] += _bd_left(KVTs[l], lambda t0, t1: DG[t0:t1, :])
        DWVT[...] += _bd_left(DKVT, lambda t0, t1: Gs[l][t0:t1, :])
        dg = _bd_left(DKV, lambda t0, t1: wvT[t0:t1, :])
        DG[...] = dg.astype(BF)
        wcat[:, 2 * D:3 * D] = dg.T.astype(BF)
        DZC[...] = jnp.broadcast_to(-jnp.sum(ZACC[...], axis=1, keepdims=True), (D, 128))

    def phase_f(l):
        def body(t, carry):
            cs = cols(t)
            nb = Ns[l][:, cs]
            dpk = _dot(DG[...], nb) + _tile_lanes(DZC[...], TS)
            pk = QKs[l][2 * D:3 * D, cs].astype(F32)
            QKs[l][D:2 * D, cs] = (dpk * jnp.minimum(pk - PEPS, 1.0)).astype(BF)
            dn = _dot(wcat[...], QKs[l][:, cs])
            DWQK[...] += _dot(nb, QKs[l][0:2 * D, cs], NT)
            n = nb.astype(F32)
            r = STAT[l:l + 1, cs]
            dx = X[:, cs] + r * (dn - _colmean(dn) - n * _colmean(dn * n))
            if l == 1:
                X[:, cs] = dx
                Y1[:, cs] = dx.astype(BF)
                GN[cs, :] = dx.T.astype(BF)
                DB2[...] += _lanesum(dx)
                DY[:, cs] = jnp.zeros((D, TS), F32)
            else:
                xin[:, cs] = dx.astype(BF)
                dx_copy(t).start()
            return carry

        lax.fori_loop(0, NTS, body, 0)

    phase_c(0)
    in_copies[1].wait()
    in_copies[2].wait()
    b2c[...] = jnp.broadcast_to(b2[...].astype(F32), (128, D)).T
    fin_fwd(0)
    phase_a(0)
    in_copies[3].wait()
    in_copies[4].wait()
    in_copies[5].wait()
    mlp_fwd()
    phase_c(1)
    fin_fwd(1)
    in_copies[6].wait()
    phase_a(1)
    mlp_fwd_bwd()
    phase_e(1)
    fin_bwd(1)
    phase_f(1)
    mlp_bwd()
    db1s[...] = jnp.sum(DB1[...], axis=0, keepdims=True).astype(BF)
    db2s[...] = jnp.sum(DB2[...].T, axis=0, keepdims=True).astype(BF)
    small = [pltpu.make_async_copy(db1s, db1_hbm, sem_out.at[0]),
             pltpu.make_async_copy(db2s, db2_hbm, sem_out.at[1]),
             pltpu.make_async_copy(wo, dwo_hbm, sem_out.at[2]),
             pltpu.make_async_copy(wqkv, dwqkv_hbm, sem_out.at[3])]
    small[0].start()
    small[1].start()
    phase_e(0)
    fin_bwd(0)
    wo[...] = DWO[...].astype(BF)
    small[2].start()
    wqkv[:, 2 * D:3 * D] = DWVT[...].T.astype(BF)
    phase_f(0)
    wqkv[:, 0:2 * D] = DWQK[...].astype(BF)
    small[3].start()
    for t in range(NTS):
        out_copy(t).wait()
    for j in range(F // TF3):
        for c in w_out_copies(j):
            c.wait()
    for t in range(NTS):
        dx_copy(t).wait()
    for c in small:
        c.wait()


@jax.jit
def pallas_interleave_layers__linear_attn_block__mixer_channel_mlp__prompt_kernel(
    A_x: jax.Array,
    A_wqkv: jax.Array,
    A_wo: jax.Array,
    B_x: jax.Array,
    B_w1: jax.Array,
    B_b1: jax.Array,
    B_w2: jax.Array,
    B_b2: jax.Array,
    grad_out: jax.Array,
):
    del B_x
    xT = jnp.swapaxes(A_x[0], 0, 1)
    gT = jnp.swapaxes(grad_out[0], 0, 1)
    V = pltpu.VMEM
    scratch = [
        V((D, S), BF), V((D, S), BF), V((D, 3 * D), BF), V((D, D), BF),
        V((D, F), BF), V((D, F), BF), V((1, F), BF), V((1, D), BF),
        V((D, S), F32), V((D, S), F32),
        V((D, S), BF), V((D, S), BF), V((D, S), BF), V((D, S), BF),
        V((3 * D, S), BF), V((3 * D, S), BF),
        V((S, F), BF), V((S, D), BF), V((S, D), BF), V((8, S), F32),
        V((2 * D, D), BF), V((D, D), BF), V((D, D), BF), V((D, 3 * D), BF),
        V((D, D), BF), V((D, 128), F32),
        V((D, D), BF), V((D, D), BF), V((D, D), BF), V((D, D), BF),
        V((D, D), BF), V((D, D), BF), V((D, D), BF), V((D, D), BF),
        V((D, D), BF), V((D, D), BF), V((D, 128), F32), V((D, 128), F32),
        V((D, D), F32), V((D, 128), F32),
        V((D, D), BF), V((D, D), BF), V((D, D), BF), V((D, 128), F32),
        V((D, F), F32), V((D, F), F32), V((8, F), F32), V((D, 128), F32),
        V((D, 2 * D), F32), V((D, D), F32), V((D, D), F32),
        V((1, F), BF), V((1, D), BF),
        pltpu.SemaphoreType.DMA((7,)), pltpu.SemaphoreType.DMA((NTS,)),
        pltpu.SemaphoreType.DMA((4,)), pltpu.SemaphoreType.DMA((NTS,)),
        pltpu.SemaphoreType.DMA((NTS,)),
        pltpu.SemaphoreType.DMA((F // TF3,)), pltpu.SemaphoreType.DMA((F // TF3,)),
    ]
    sds = jax.ShapeDtypeStruct
    outT, dxT, dwqkv, dwo, dw1, db1, dw2T, db2 = pl.pallas_call(
        _kernel,
        in_specs=[pl.BlockSpec(memory_space=pl.ANY)] * 8,
        out_specs=[pl.BlockSpec(memory_space=pl.ANY)] * 8,
        out_shape=[sds((D, S), BF), sds((D, S), BF), sds((D, 3 * D), BF), sds((D, D), BF),
                   sds((D, F), BF), sds((1, F), BF), sds((D, F), BF), sds((1, D), BF)],
        scratch_shapes=scratch,
        compiler_params=pltpu.CompilerParams(vmem_limit_bytes=128 * 2**20),
    )(xT, gT, A_wqkv, A_wo, B_w1, B_b1.reshape(1, F), B_w2.T, B_b2.reshape(1, D))
    return (jnp.swapaxes(outT, 0, 1)[None], jnp.swapaxes(dxT, 0, 1)[None], dwqkv, dwo, dw1,
            db1.reshape(F), dw2T.T, db2.reshape(D))
```

```python
import functools

import jax
import jax.numpy as jnp
from jax import lax
import jax.experimental.pallas as pl
import jax.experimental.pallas.tpu as pltpu

S, D, F, H, DH = 2048, 576, 4608, 32, 18
HS, HD = S // 2, D // 2
EPS = 1e-5
PEPS = 1e-6
BF = jnp.bfloat16
F32 = jnp.float32
NN = (((1,), (0,)), ((), ()))
NT = (((1,), (1,)), ((), ()))
C0 = 0.7978845608028654
C1 = 0.7978845608028654 * 0.044715

PIECES = ((0, 144, 0, 128), (112, 272, 128, 256), (240, 400, 256, 384), (368, 528, 384, 512),
          (496, 576, 512, 576))

TH = 256
TS = 2 * TH
NTS = HS // TH
T1 = 256
T2 = 128
NC1 = F // (2 * T1)
NC2 = F // (2 * T2)
RB1 = 64
RB = 16
KW = (320, 320, 320, 256, 256, 320, 256)
A2B = (0, 6, 1, 4, 5, 3, 2)
SCOPES = False


ONLY = None


def _scoped(name, fn, *args):
    if ONLY is not None and name not in ONLY:
        return None
    if SCOPES:
        with jax.named_scope(name):
            return fn(*args)
    return fn(*args)


def _dot(a, b, dn=NN):
    return lax.dot_general(a, b, dn, preferred_element_type=F32)


def _assemble(ps):
    segs = []
    for j, (r0, r1, _, _) in enumerate(PIECES):
        lo = r0 if j == 0 else PIECES[j - 1][1]
        hi = r1 if j == len(PIECES) - 1 else PIECES[j + 1][0]
        segs.append(ps[j][lo - r0:hi - r0])
        if j != len(PIECES) - 1:
            segs.append(ps[j][hi - r0:r1 - r0] + ps[j + 1][0:r1 - hi])
    return jnp.concatenate(segs, axis=0)


def _bd_left(bd_ref, rhs_rows):
    return _assemble([_dot(bd_ref[j, 0:r1 - r0, 0:t1 - t0], rhs_rows(t0, t1))
                      for j, (r0, r1, t0, t1) in enumerate(PIECES)])


def _lanesum(a):
    acc = a[:, 0:128]
    for i in range(1, a.shape[1] // 128):
        acc = acc + a[:, i * 128:(i + 1) * 128]
    return acc


def _tile_lanes(col128, n):
    return col128 if n == 128 else jnp.concatenate([col128] * (n // 128), axis=1)


def _colmean(a):
    return jnp.sum(a, axis=0, keepdims=True) * (1.0 / D)


def _gelu(x, with_grad):
    u = x * x
    s = 0.5 + 0.5 * jnp.tanh(x * (C0 + C1 * u))
    h = x * s
    if not with_grad:
        return h, None
    return h, s + h * (1.0 - s) * (2.0 * C0 + (6.0 * C1) * u)


def _recomb(m):
    return (m[0] + m[3] - m[4] + m[6], m[2] + m[4], m[1] + m[3], m[0] - m[1] + m[2] + m[5])


def _bcombos(b11, b12, b21, b22):
    return (b11 + b22, b11, b12 - b22, b21 - b11, b22, b11 + b12, b21 + b22)


def _acombos(a11, a12, a21, a22):
    return (a11 + a22, a21 + a22, a11, a22, a11 + a12, a21 - a11, a12 - a22)


def _store_wk(dst, w, fa, fb):
    c = _bcombos(w[0:256, fa].astype(F32), w[0:256, fb].astype(F32),
                 w[256:512, fa].astype(F32), w[256:512, fb].astype(F32))
    for i in range(7):
        dst[i, 0:256, :] = c[i].astype(BF)
    ra, rb = w[512:D, fa], w[512:D, fb]
    dst[0, 256:320, :] = ra
    dst[1, 256:320, :] = ra
    dst[2, 256:320, :] = rb
    dst[5, 256:320, :] = (ra.astype(F32) + rb.astype(F32)).astype(BF)


def _store_wm(dst, w, fa, fb):
    c = _acombos(w[0:HD, fa].astype(F32), w[0:HD, fb].astype(F32),
                 w[HD:D, fa].astype(F32), w[HD:D, fb].astype(F32))
    for i in range(7):
        dst[i] = c[i].astype(BF)


def _store_nat(dst, rows, v):
    n1, n2 = v[:, 0:TH].T, v[:, TH:TS].T
    c = _acombos(n1[:, 0:256], n1[:, 256:512], n2[:, 0:256], n2[:, 256:512])
    for i in range(7):
        dst[i, rows, 0:256] = c[i].astype(BF)
    r1, r2 = n1[:, 512:D], n2[:, 512:D]
    dst[0, rows, 256:320] = r1.astype(BF)
    dst[1, rows, 256:320] = r2.astype(BF)
    dst[2, rows, 256:320] = r1.astype(BF)
    dst[5, rows, 256:320] = (r2 - r1).astype(BF)


def _store_tc(dst, cols, v):
    c = _bcombos(v[0:HD, 0:TH], v[HD:D, 0:TH], v[0:HD, TH:TS], v[HD:D, TH:TS])
    for k, i in enumerate((0, 2, 3, 5, 6)):
        dst[k, :, cols] = c[i].astype(BF)


def _tc_operand(comb, plain, i):
    if i == 1:
        return plain[0:HD, 0:HS]
    if i == 4:
        return plain[HD:D, HS:S]
    return comb[(0, None, 1, 2, None, 3, 4)[i]]


def _kernel(x_hbm, g_hbm, wqkv_hbm, wo_hbm, w1_hbm, b1_hbm, w2_hbm, b2_hbm,
            out_hbm, dx_hbm, dwqkv_hbm, dwo_hbm, dw1_hbm, db1_hbm, dw2_hbm, db2_hbm, pre_hbm,
            gin, wcat, wo, w1, w2, b1, b2,
            X, OA, DA, N0, N1, Y0, Y1, QK0, QK1, STAT,
            YA, GA, YC, GC, HC1, HC, DC, WBa, WAa, WB1, WB2, WA1, WA2, PST1, PST,
            wqkT, wv, wvT, bmask, b2c,
            G0, G1, KV, KVT0, KVT1, M0, M1, MT, ZM, ZC0, ZC1,
            ACC, ZACC, DG, DKV, DKVT, DZC,
            DW1, DW2, DB1, DB2, DWQK, DWVT, DWO, db1s, db2s,
            sem_in, sem_x, sem_out, sem_o, sem_dx, sem_w1, sem_w2, sem_ps, sem_pl):
    Ns, Ys, QKs = (N0, N1), (Y0, Y1), (QK0, QK1)
    Gs, KVTs, Ms, ZCs = (G0, G1), (KVT0, KVT1), (M0, M1), (ZC0, ZC1)
    xin = N1

    def cols(t):
        return pl.ds(pl.multiple_of(t * TS, TS), TS)

    def half(t, h):
        return pl.ds(pl.multiple_of(h * HS + t * TH, TH), TH)

    def ld2(ref, t):
        return jnp.concatenate([ref[:, half(t, 0)], ref[:, half(t, 1)]], axis=1)

    def st2(ref, t, v):
        ref[:, half(t, 0)] = v[:, 0:TH]
        ref[:, half(t, 1)] = v[:, TH:TS]

    def recomb_tile(acc, nacc, t):
        m = [acc[i, :, half(t, 0)] for i in range(nacc)]
        c11 = m[0] + m[3] - m[4]
        c22 = m[0] - m[1] + m[2]
        if nacc == 7:
            c11 = c11 + m[6]
            c22 = c22 + m[5]
        return jnp.concatenate([jnp.concatenate([c11, m[2] + m[4]], axis=1),
                                jnp.concatenate([m[1] + m[3], c22], axis=1)], axis=0)

    def zero_acc(acc, nacc, t):
        for i in range(nacc):
            acc[i, :, half(t, 0)] = jnp.zeros((HD, TH), F32)

    def x_copy(t, h):
        return pltpu.make_async_copy(x_hbm.at[:, half(t, h)], xin.at[:, half(t, h)],
                                     sem_x.at[2 * t + h])

    in_copies = [
        pltpu.make_async_copy(wqkv_hbm, wcat, sem_in.at[0]),
        pltpu.make_async_copy(wo_hbm, wo, sem_in.at[1]),
        pltpu.make_async_copy(b2_hbm, b2, sem_in.at[2]),
        pltpu.make_async_copy(b1_hbm, b1, sem_in.at[3]),
        pltpu.make_async_copy(w1_hbm, w1, sem_in.at[4]),
        pltpu.make_async_copy(w2_hbm, w2, sem_in.at[5]),
        pltpu.make_async_copy(g_hbm, gin, sem_in.at[6]),
    ]
    in_copies[0].start()
    for t in range(NTS):
        x_copy(t, 0).start()
        x_copy(t, 1).start()
    for c in in_copies[1:]:
        c.start()

    for j, (r0, r1, t0, t1) in enumerate(PIECES):
        ri = (lax.broadcasted_iota(jnp.int32, (160, 128), 0) + r0).astype(F32)
        ci = (lax.broadcasted_iota(jnp.int32, (160, 128), 1) + t0).astype(F32)
        same = jnp.floor((ri + 0.5) * (1.0 / DH)) == jnp.floor((ci + 0.5) * (1.0 / DH))
        bmask[j] = jnp.where(same, 1.0, 0.0).astype(BF)
    DWQK[...] = jnp.zeros(DWQK.shape, F32)
    DWVT[...] = jnp.zeros(DWVT.shape, F32)
    DWO[...] = jnp.zeros(DWO.shape, F32)
    DB2[...] = jnp.zeros(DB2.shape, F32)

    in_copies[0].wait()
    wqkT[...] = wcat[:, 0:2 * D].astype(F32).T.astype(BF)
    wvv = wcat[:, 2 * D:3 * D]
    wv[...] = wvv
    wvT[...] = wvv.astype(F32).T.astype(BF)

    def phase_c(l):
        ACC[...] = jnp.zeros(ACC.shape, F32)
        ZACC[...] = jnp.zeros(ZACC.shape, F32)

        def body(t, carry):
            cs = cols(t)
            if l == 0:
                x_copy(t, 0).wait()
                x_copy(t, 1).wait()
                x = ld2(xin, t).astype(F32)
            else:
                x = ld2(X, t) + recomb_tile(OA, 5, t)
            st2(X, t, x)
            c = x - _colmean(x)
            r = lax.rsqrt(_colmean(c * c) + EPS)
            n = (c * r).astype(BF)
            Ns[l][:, cs] = n
            STAT[l:l + 1, cs] = r
            qk = _dot(wqkT[...], n)
            ph = jnp.where(qk > 0, qk + 1.0, jnp.exp(jnp.minimum(qk, 0.0))) + PEPS
            QKs[l][0:D, cs] = ph[0:D].astype(BF)
            pk = ph[D:2 * D]
            pkb = pk.astype(BF)
            QKs[l][2 * D:3 * D, cs] = pkb
            ACC[...] += _dot(pkb, n, NT)
            ZACC[...] += _lanesum(pk)
            return carry

        lax.fori_loop(0, NTS, body, 0)

    def fin_fwd(l):
        Gs[l][...] = ACC[...].astype(BF)
        za = ZACC[...]
        zrow = jnp.sum(za.T, axis=0, keepdims=True)
        for j, (r0, r1, t0, t1) in enumerate(PIECES):
            mk = bmask[j, 0:r1 - r0, 0:t1 - t0].astype(F32)
            KV[j, 0:r1 - r0, 0:t1 - t0] = (_dot(Gs[l][r0:r1, :], wv[:, t0:t1]) * mk).astype(BF)
            KVTs[l][j, 0:r1 - r0, 0:t1 - t0] = (
                _dot(wvT[r0:r1, :], Gs[l][t0:t1, :], NT) * mk).astype(BF)
            ZM[j, 0:r1 - r0, 0:t1 - t0] = (mk * zrow[:, t0:t1]).astype(BF)
        m = _bd_left(KV, lambda t0, t1: wo[t0:t1, :])
        Ms[l][...] = m.astype(BF)
        MT[...] = m.T.astype(BF)
        ZCs[l][...] = jnp.broadcast_to(jnp.sum(za, axis=1, keepdims=True), (D, 128))

    def phase_a(l):
        def body(t, carry):
            cs = cols(t)
            den = _bd_left(ZM, lambda t0, t1: QKs[l][t0:t1, cs]) + PEPS
            rden = pl.reciprocal(den, approx=True)
            rden = rden * (2.0 - den * rden)
            pq = QKs[l][0:D, cs].astype(F32)
            p = (pq * rden).astype(BF)
            QKs[l][D:2 * D, cs] = p
            QKs[l][0:D, cs] = (rden * jnp.minimum(pq - PEPS, 1.0)).astype(BF)
            x = ld2(X, t) + _dot(MT[...], p)
            c = x - _colmean(x)
            s = lax.rsqrt((1.0 + EPS) * _colmean(c * c) + EPS * EPS)
            y = c * s
            st2(Ys[l], t, y.astype(BF))
            STAT[2 + l:3 + l, cs] = s
            _store_nat(YA, half(t, 0), y)
            st2(X, t, x + _tile_lanes(b2c[...], TS))
            zero_acc(OA, 5, t)
            if l == 1:
                _store_tc(YC, half(t, 0), y)
                g = ld2(gin, t).astype(F32)
                _store_nat(GA, half(t, 0), g)
                _store_tc(GC, half(t, 0), g)
                DB2[...] += _lanesum(g)
                zero_acc(DA, 7, t)
            return carry

        lax.fori_loop(0, NTS, body, 0)

    def chunk(j, tw):
        return (pl.ds(pl.multiple_of(j * 2 * tw, tw), tw),
                pl.ds(pl.multiple_of(j * 2 * tw + tw, tw), tw))

    def out_acc(i, r0, v):
        if i == 6:
            X[0:HD, r0:r0 + 128] += v
        elif i == 5:
            X[HD:D, HS + r0:HS + r0 + 128] += v
        else:
            OA[i, :, r0:r0 + 128] += v

    NPC = T1 // T2

    def pre_store_copy(j, k):
        return pltpu.make_async_copy(PST1.at[j % 2, :, pl.ds(k * 2 * T2, 2 * T2)],
                                     pre_hbm.at[j * NPC + k], sem_ps.at[j * NPC + k])

    def pre_load_copy(j):
        return pltpu.make_async_copy(pre_hbm.at[j], PST.at[j % 2], sem_pl.at[j])

    def mlp_fwd():
        fa, fb = chunk(0, T1)
        _store_wk(WBa, w1, fa, fb)
        _store_wm(WAa, w2, fa, fb)

        def body(j, carry):
            @pl.when(j >= 2)
            def _():
                for k in range(NPC):
                    pre_store_copy(j - 2, k).wait()

            @pl.when(j >= 1)
            def _():
                for k in range(NPC):
                    pre_store_copy(j - 1, k).start()

            fa, fb = chunk(j, T1)
            sl = j % 2
            bias = (b1[:, fa].astype(F32), b1[:, fb].astype(F32))
            jobs = []

            def j_oa(i, r0):
                out_acc(i, r0, _dot(WAa[i], HC1[i, r0:r0 + 128, :], NT))

            per = -(-7 * RB1 // 128)
            for r0 in range(0, HS, RB1):
                P = [_dot(YA[i, r0:r0 + RB1, 0:KW[i]], WBa[i, 0:KW[i], :]) for i in range(7)]
                if r0 >= 128 and r0 % 128 == 0:
                    jobs += [functools.partial(j_oa, i, r0 - 128) for i in range(7)]
                for _ in range(per):
                    if jobs:
                        jobs.pop(0)()
                for r in range(0, RB1, RB):
                    pre = _recomb([p[r:r + RB] for p in P])
                    pre = [pre[q] + bias[q % 2] for q in range(4)]
                    for q in range(4):
                        rr = (q // 2) * HS + r0 + r
                        PST1[sl, rr:rr + RB, (q % 2) * T1:(q % 2 + 1) * T1] = pre[q].astype(BF)
                    hh = [_gelu(v, False)[0] for v in pre]
                    hc = _bcombos(hh[0], hh[2], hh[1], hh[3])
                    for i in range(7):
                        HC1[i, r0 + r:r0 + r + RB, :] = hc[i].astype(BF)
            na, nb = chunk(jnp.minimum(j + 1, NC1 - 1), T1)
            _store_wk(WBa, w1, na, nb)
            jobs += [functools.partial(j_oa, i, HS - 128) for i in range(7)]
            while jobs:
                jobs.pop(0)()
            _store_wm(WAa, w2, na, nb)
            return carry

        lax.fori_loop(0, NC1, body, 0)
        for k in range(NPC):
            pre_store_copy(NC1 - 1, k).start()
        for k in range(NPC):
            pre_store_copy(NC1 - 2, k).wait()

    def w_out_copies(j):
        fc = pl.ds(pl.multiple_of(j * 2 * T2, 2 * T2), 2 * T2)
        return (pltpu.make_async_copy(DW1.at[:, fc], dw1_hbm.at[:, fc], sem_w1.at[j]),
                pltpu.make_async_copy(DW2.at[:, fc], dw2_hbm.at[:, fc], sem_w2.at[j]))

    def mlp_bwd(l):
        gplain = gin if l == 1 else Y1
        fa, fb = chunk(0, T2)
        _store_wk(WB2, w2, fa, fb)
        _store_wm(WA1, w1, fa, fb)
        if l == 1:
            _store_wk(WB1, w1, fa, fb)
            _store_wm(WA2, w2, fa, fb)

        def body(j, carry):
            if l == 0:
                pre_load_copy(j).wait()

                @pl.when(j + 1 < NC2)
                def _():
                    pre_load_copy(j + 1).start()

                @pl.when(j >= 1)
                def _():
                    for c in w_out_copies(j - 1):
                        c.start()

            fa, fb = chunk(j, T2)
            sl = j % 2
            if l == 1:
                bias = (b1[:, fa].astype(F32), b1[:, fb].astype(F32))
            jobs = []

            def j_oa(i, r0):
                out_acc(i, r0, _dot(WA2[i], HC[i, r0:r0 + 128, :], NT))

            def j_da(i, r0):
                DA[i, :, r0:r0 + 128] += _dot(WA1[i], DC[i, r0:r0 + 128, :], NT)

            def add_jobs(r0):
                for i in range(7):
                    if l == 1:
                        jobs.append(functools.partial(j_oa, i, r0))
                    jobs.append(functools.partial(j_da, i, r0))

            def dw(dst, comb, plain, src):
                c = _recomb([_dot(_tc_operand(comb, plain, i), src[A2B[i]]) for i in range(7)])
                for q, (rs, fs) in enumerate(((0, fa), (HD, fa), (0, fb), (HD, fb))):
                    v = c[q]
                    if l == 0:
                        v = v + dst[rs:rs + HD, fs].astype(F32)
                    dst[rs:rs + HD, fs] = v.astype(BF)

            per = -(-(14 if l == 1 else 7) * RB1 // 128)
            sa = jnp.zeros((8, T2), F32)
            sb = jnp.zeros((8, T2), F32)
            for r0 in range(0, HS, RB1):
                if l == 1:
                    P = [_dot(YA[i, r0:r0 + RB1, 0:KW[i]], WB1[i, 0:KW[i], :]) for i in range(7)]
                Q = [_dot(GA[i, r0:r0 + RB1, 0:KW[i]], WB2[i, 0:KW[i], :]) for i in range(7)]
                if r0 >= 128 and r0 % 128 == 0:
                    add_jobs(r0 - 128)
                for _ in range(per):
                    if jobs:
                        jobs.pop(0)()
                for r in range(0, RB1, RB):
                    if l == 1:
                        pre = _recomb([p[r:r + RB] for p in P])
                        pre = [pre[q] + bias[q % 2] for q in range(4)]
                    else:
                        pre = [PST[sl, (q // 2) * HS + r0 + r:(q // 2) * HS + r0 + r + RB,
                                   (q % 2) * T2:(q % 2 + 1) * T2].astype(F32) for q in range(4)]
                    dh = _recomb([p[r:r + RB] for p in Q])
                    hg = [_gelu(v, True) for v in pre]
                    hc = _bcombos(hg[0][0], hg[2][0], hg[1][0], hg[3][0])
                    dp = [dh[q] * hg[q][1] for q in range(4)]
                    dc = _bcombos(dp[0], dp[2], dp[1], dp[3])
                    sa = sa + jnp.sum(dc[5].reshape(RB // 8, 8, T2), axis=0)
                    sb = sb + jnp.sum(dc[6].reshape(RB // 8, 8, T2), axis=0)
                    for i in range(7):
                        HC[i, r0 + r:r0 + r + RB, :] = hc[i].astype(BF)
                        DC[i, r0 + r:r0 + r + RB, :] = dc[i].astype(BF)
            if l == 1:
                DB1[:, fa] = sa
                DB1[:, fb] = sb
            else:
                DB1[:, fa] += sa
                DB1[:, fb] += sb
            na, nb = chunk(jnp.minimum(j + 1, NC2 - 1), T2)
            dw(DW2, GC, gplain, HC)
            _store_wk(WB2, w2, na, nb)
            if l == 1:
                _store_wk(WB1, w1, na, nb)
            add_jobs(HS - 128)
            while jobs:
                jobs.pop(0)()
            dw(DW1, YC, Ys[l], DC)
            _store_wm(WA1, w1, na, nb)
            if l == 1:
                _store_wm(WA2, w2, na, nb)
            return carry

        lax.fori_loop(0, NC2, body, 0)
        if l == 0:
            for c in w_out_copies(NC2 - 1):
                c.start()

    def out_copy(t, h):
        return pltpu.make_async_copy(gin.at[:, half(t, h)], out_hbm.at[:, half(t, h)],
                                     sem_o.at[2 * t + h])

    def dx_copy(t, h):
        return pltpu.make_async_copy(xin.at[:, half(t, h)], dx_hbm.at[:, half(t, h)],
                                     sem_dx.at[2 * t + h])

    def phase_e(l):
        ACC[...] = jnp.zeros(ACC.shape, F32)
        ZACC[...] = jnp.zeros(ZACC.shape, F32)

        def body(t, carry):
            cs = cols(t)
            if l == 1:
                g = ld2(gin, t).astype(F32)
                st2(gin, t, (ld2(X, t) + recomb_tile(OA, 5, t)).astype(BF))
                out_copy(t, 0).start()
                out_copy(t, 1).start()
            else:
                g = ld2(X, t)
            y = ld2(Ys[l], t).astype(F32)
            dy = recomb_tile(DA, 7, t)
            s = STAT[2 + l:3 + l, cs]
            dx = g + s * (dy - _colmean(dy) - y * ((1.0 + EPS) * _colmean(dy * y)))
            st2(X, t, dx)
            dxb = dx.astype(BF)
            dp = _dot(Ms[l][...], dxb)
            pb = QKs[l][D:2 * D, cs]
            ACC[...] += _dot(pb, dxb, NT)
            p = pb.astype(F32)
            tt = (dp * p).astype(BF)
            hs = _bd_left(bmask, lambda t0, t1: tt[t0:t1])
            cq = QKs[l][0:D, cs].astype(F32)
            QKs[l][0:D, cs] = (cq * (dp - _tile_lanes(ZCs[l][...], TS) * hs)).astype(BF)
            ZACC[...] += _lanesum(p * hs)
            return carry

        lax.fori_loop(0, NTS, body, 0)

    def fin_bwd(l):
        DG[...] = ACC[...].astype(BF)
        for j, (r0, r1, t0, t1) in enumerate(PIECES):
            mk = bmask[j, 0:r1 - r0, 0:t1 - t0].astype(F32)
            DKV[j, 0:r1 - r0, 0:t1 - t0] = (_dot(DG[r0:r1, :], wo[t0:t1, :], NT) * mk).astype(BF)
            DKVT[j, 0:r1 - r0, 0:t1 - t0] = (_dot(wo[r0:r1, :], DG[t0:t1, :], NT) * mk).astype(BF)
        DWO[...] += _bd_left(KVTs[l], lambda t0, t1: DG[t0:t1, :])
        DWVT[...] += _bd_left(DKVT, lambda t0, t1: Gs[l][t0:t1, :])
        dg = _bd_left(DKV, lambda t0, t1: wvT[t0:t1, :])
        DG[...] = dg.astype(BF)
        wcat[:, 2 * D:3 * D] = dg.T.astype(BF)
        DZC[...] = jnp.broadcast_to(-jnp.sum(ZACC[...], axis=1, keepdims=True), (D, 128))

    def phase_f(l):
        def body(t, carry):
            cs = cols(t)
            nb = Ns[l][:, cs]
            dpk = _dot(DG[...], nb) + _tile_lanes(DZC[...], TS)
            pk = QKs[l][2 * D:3 * D, cs].astype(F32)
            QKs[l][D:2 * D, cs] = (dpk * jnp.minimum(pk - PEPS, 1.0)).astype(BF)
            dn = _dot(wcat[...], QKs[l][:, cs])
            DWQK[...] += _dot(nb, QKs[l][0:2 * D, cs], NT)
            n = nb.astype(F32)
            r = STAT[l:l + 1, cs]
            dx = ld2(X, t) + r * (dn - _colmean(dn) - n * _colmean(dn * n))
            if l == 1:
                st2(X, t, dx)
                st2(Y1, t, dx.astype(BF))
                _store_nat(GA, half(t, 0), dx)
                _store_tc(GC, half(t, 0), dx)
                _store_tc(YC, half(t, 0), ld2(Y0, t).astype(F32))
                DB2[...] += _lanesum(dx)
                zero_acc(DA, 7, t)
            else:
                st2(xin, t, dx.astype(BF))
                dx_copy(t, 0).start()
                dx_copy(t, 1).start()
            return carry

        lax.fori_loop(0, NTS, body, 0)

    _scoped('phase_c0', phase_c, 0)
    in_copies[1].wait()
    in_copies[2].wait()
    b2c[...] = jnp.broadcast_to(b2[...].astype(F32), (128, D)).T
    _scoped('fin_fwd0', fin_fwd, 0)
    _scoped('phase_a0', phase_a, 0)
    in_copies[3].wait()
    in_copies[4].wait()
    in_copies[5].wait()
    _scoped('mlp_fwd', mlp_fwd)
    _scoped('phase_c1', phase_c, 1)
    for k in range(NPC):
        pre_store_copy(NC1 - 1, k).wait()
    _scoped('fin_fwd1', fin_fwd, 1)
    in_copies[6].wait()
    _scoped('phase_a1', phase_a, 1)
    _scoped('mlp_bwd1', mlp_bwd, 1)
    _scoped('phase_e1', phase_e, 1)
    _scoped('fin_bwd1', fin_bwd, 1)
    pre_load_copy(0).start()
    _scoped('phase_f1', phase_f, 1)
    _scoped('mlp_bwd0', mlp_bwd, 0)
    db1s[...] = jnp.sum(DB1[...], axis=0, keepdims=True).astype(BF)
    db2s[...] = jnp.sum(DB2[...].T, axis=0, keepdims=True).astype(BF)
    small = [pltpu.make_async_copy(db1s, db1_hbm, sem_out.at[0]),
             pltpu.make_async_copy(db2s, db2_hbm, sem_out.at[1]),
             pltpu.make_async_copy(wo, dwo_hbm, sem_out.at[2]),
             pltpu.make_async_copy(wv, dwqkv_hbm.at[:, pl.ds(2 * D, D)], sem_out.at[3]),
             pltpu.make_async_copy(wcat.at[:, pl.ds(0, 2 * D)], dwqkv_hbm.at[:, pl.ds(0, 2 * D)],
                                   sem_out.at[4])]
    small[0].start()
    small[1].start()
    _scoped('phase_e0', phase_e, 0)
    _scoped('fin_bwd0', fin_bwd, 0)
    wo[...] = DWO[...].astype(BF)
    small[2].start()
    wv[...] = DWVT[...].T.astype(BF)
    small[3].start()
    _scoped('phase_f0', phase_f, 0)
    wcat[:, 0:2 * D] = DWQK[...].astype(BF)
    small[4].start()
    for t in range(NTS):
        out_copy(t, 0).wait()
        out_copy(t, 1).wait()
    for j in range(NC2):
        for c in w_out_copies(j):
            c.wait()
    for t in range(NTS):
        dx_copy(t, 0).wait()
        dx_copy(t, 1).wait()
    for c in small:
        c.wait()


@jax.jit
def pallas_interleave_layers__linear_attn_block__mixer_channel_mlp__prompt_kernel(
    A_x: jax.Array,
    A_wqkv: jax.Array,
    A_wo: jax.Array,
    B_x: jax.Array,
    B_w1: jax.Array,
    B_b1: jax.Array,
    B_w2: jax.Array,
    B_b2: jax.Array,
    grad_out: jax.Array,
):
    del B_x
    xT = jnp.swapaxes(A_x[0], 0, 1)
    gT = jnp.swapaxes(grad_out[0], 0, 1)
    V = pltpu.VMEM
    PC = V((5, 160, 128), BF)
    DD = V((D, D), BF)
    COL = V((D, 128), F32)
    DSB = V((D, S), BF)
    scratch = [
        DSB, V((D, 3 * D), BF), DD, V((D, F), BF), V((D, F), BF), V((1, F), BF), V((1, D), BF),
        V((D, S), F32), V((5, HD, HS), F32), V((7, HD, HS), F32),
        DSB, DSB, DSB, DSB, V((3 * D, S), BF), V((3 * D, S), BF), V((8, S), F32),
        V((7, HS, 384), BF), V((7, HS, 384), BF),
        V((5, HD, HS), BF), V((5, HD, HS), BF),
        V((7, HS, T1), BF), V((7, HS, T2), BF), V((7, HS, T2), BF),
        V((7, 320, T1), BF), V((7, HD, T1), BF),
        V((7, 320, T2), BF), V((7, 320, T2), BF), V((7, HD, T2), BF), V((7, HD, T2), BF),
        V((2, S, 2 * T1), BF), V((2, S, 2 * T2), BF),
        V((2 * D, D), BF), DD, DD, PC, COL,
        DD, DD, PC, PC, PC, DD, DD, DD, PC, COL, COL,
        V((D, D), F32), COL, DD, PC, PC, COL,
        V((D, F), BF), V((D, F), BF), V((8, F), F32), COL,
        V((D, 2 * D), F32), V((D, D), F32), V((D, D), F32),
        V((1, F), BF), V((1, D), BF),
        pltpu.SemaphoreType.DMA((7,)), pltpu.SemaphoreType.DMA((2 * NTS,)),
        pltpu.SemaphoreType.DMA((5,)), pltpu.SemaphoreType.DMA((2 * NTS,)),
        pltpu.SemaphoreType.DMA((2 * NTS,)),
        pltpu.SemaphoreType.DMA((NC2,)), pltpu.SemaphoreType.DMA((NC2,)),
        pltpu.SemaphoreType.DMA((NC2,)), pltpu.SemaphoreType.DMA((NC2,)),
    ]
    sds = jax.ShapeDtypeStruct
    outT, dxT, dwqkv, dwo, dw1, db1, dw2T, db2, _ = pl.pallas_call(
        _kernel,
        in_specs=[pl.BlockSpec(memory_space=pl.ANY)] * 8,
        out_specs=[pl.BlockSpec(memory_space=pl.ANY)] * 9,
        out_shape=[sds((D, S), BF), sds((D, S), BF), sds((D, 3 * D), BF), sds((D, D), BF),
                   sds((D, F), BF), sds((1, F), BF), sds((D, F), BF), sds((1, D), BF),
                   sds((NC2, S, 2 * T2), BF)],
        scratch_shapes=scratch,
        compiler_params=pltpu.CompilerParams(vmem_limit_bytes=128 * 2**20),
    )(xT, gT, A_wqkv, A_wo, B_w1, B_b1.reshape(1, F), B_w2.T, B_b2.reshape(1, D))
    return (jnp.swapaxes(outT, 0, 1)[None], jnp.swapaxes(dxT, 0, 1)[None], dwqkv, dwo, dw1,
            db1.reshape(F), dw2T.T, db2.reshape(D))
```

```python
import functools

import jax
import jax.numpy as jnp
from jax import lax
import jax.experimental.pallas as pl
import jax.experimental.pallas.tpu as pltpu

S, D, F, H, DH = 2048, 576, 4608, 32, 18
HS, HD = S // 2, D // 2
EPS = 1e-5
PEPS = 1e-6
BF = jnp.bfloat16
F32 = jnp.float32
U32 = jnp.uint32
NN = (((1,), (0,)), ((), ()))
NT = (((1,), (1,)), ((), ()))
C0 = 0.7978845608028654
C1 = 0.7978845608028654 * 0.044715

PIECES = ((0, 144, 0, 128), (112, 272, 128, 256), (240, 400, 256, 384), (368, 528, 384, 512),
          (496, 576, 512, 576))

L = 128
NS = HS // L
QD = D // 4
T1 = 256
NC = F // (2 * T1)
NQ = NS // 2
R1 = 32
RB = 16
KW = (320, 320, 320, 256, 256, 320, 256)
A2B = (0, 6, 1, 4, 5, 3, 2)
FILL = (2, 1, 1, 1)
PRO = ((10, 2, 12), (14, 1, 12))
SCOPES = False


def _scoped(name, fn, *args):
    if SCOPES:
        with jax.named_scope(name):
            return fn(*args)
    return fn(*args)


class _Rows:
    def __init__(self, ds):
        self.ds = ds


class _Pk:
    def __init__(self, ref):
        self.ref = ref

    def _ix(self, idx):
        nd = len(self.ref.shape)
        if idx is Ellipsis:
            return idx
        idx = list(idx) if isinstance(idx, tuple) else [idx]
        idx = idx + [slice(None)] * (nd - len(idx))
        r = idx[nd - 2]
        if isinstance(r, _Rows):
            idx[nd - 2] = r.ds
        elif r.start is not None:
            assert r.start % 16 == 0 and r.stop % 16 == 0
            idx[nd - 2] = slice(r.start // 2, r.stop // 2)
        return tuple(idx)

    def __getitem__(self, idx):
        return pltpu.bitcast(self.ref[self._ix(idx)], BF)

    def __setitem__(self, idx, v):
        self.ref[self._ix(idx)] = pltpu.bitcast(v, U32)


def _dot(a, b, dn=NN):
    return lax.dot_general(a, b, dn, preferred_element_type=F32)


def _cat(xs, axis=1):
    return jnp.concatenate(list(xs), axis=axis)


def _assemble(ps):
    segs = []
    for j, (r0, r1, _, _) in enumerate(PIECES):
        lo = r0 if j == 0 else PIECES[j - 1][1]
        hi = r1 if j == len(PIECES) - 1 else PIECES[j + 1][0]
        segs.append(ps[j][lo - r0:hi - r0])
        if j != len(PIECES) - 1:
            segs.append(ps[j][hi - r0:r1 - r0] + ps[j + 1][0:r1 - hi])
    return _cat(segs, 0)


def _bd_left(bd_ref, rhs_rows):
    return _assemble([_dot(bd_ref[j, 0:r1 - r0, 0:t1 - t0], rhs_rows(t0, t1))
                      for j, (r0, r1, t0, t1) in enumerate(PIECES)])


def _colmean(a):
    return jnp.sum(a, axis=0, keepdims=True) * (1.0 / D)


def _gelu(x, with_grad):
    u = x * x
    s = 0.5 + 0.5 * jnp.tanh(x * (C0 + C1 * u))
    h = x * s
    if not with_grad:
        return h, None
    return h, s + h * (1.0 - s) * (2.0 * C0 + (6.0 * C1) * u)


def _recomb(m):
    return (m[0] + m[3] - m[4] + m[6], m[2] + m[4], m[1] + m[3], m[0] - m[1] + m[2] + m[5])


def _bcombos(b11, b12, b21, b22):
    return (b11 + b22, b11, b12 - b22, b21 - b11, b22, b11 + b12, b21 + b22)


def _acombos(a11, a12, a21, a22):
    return (a11 + a22, a21 + a22, a11, a22, a11 + a12, a21 - a11, a12 - a22)


_BC = ((0, 3, 1), (0, None, 0), (1, 3, -1), (2, 0, -1), (3, None, 0), (0, 1, 1), (2, 3, 1))
_AC = ((0, 3, 1), (2, 3, 1), (0, None, 0), (3, None, 0), (0, 1, 1), (2, 0, -1), (1, 3, -1))


def _combo(tab, k, b):
    x, y, sg = tab[k]
    return b[x] if sg == 0 else b[x] + b[y] if sg > 0 else b[x] - b[y]


def _combos2(tab, blk, emit, inner=range(7), plain=()):
    for o in range(7):
        oc = [_combo(tab, o, [blk[q][r] for q in range(4)]) for r in range(4)]
        for i in inner:
            emit(o, i, _combo(tab, i, oc))
        for r in plain:
            emit(o, 7 + r, oc[r])


def _hix(o, i):
    r = {1: 0, 4: 3}.get(i, i - 7)
    return 4 * o + r if r >= 0 else 28 + 5 * o + (0, 2, 3, 5, 6).index(i)


def _token(v):
    v = functools.reduce(jnp.maximum, [v[:, c:c + L] for c in range(0, v.shape[1], L)])
    return jnp.max(v.reshape(v.shape[0] // 8, 8, L), axis=0)


def _store_wk(dst, wa, wb):
    def main(r0, n):
        c = _bcombos(*[f(k + r0, k + r0 + n).astype(F32) for k in (0, 256) for f in (wa, wb)])
        for i in range(7):
            dst[i, r0:r0 + n, :] = c[i].astype(BF)
        return _token(jnp.maximum(c[5], c[6]))

    def rest():
        ra, rb = wa(512, D), wb(512, D)
        dst[0, 256:320, :] = ra
        dst[1, 256:320, :] = ra
        dst[2, 256:320, :] = rb
        dst[5, 256:320, :] = (ra.astype(F32) + rb.astype(F32)).astype(BF)

    return [functools.partial(main, r0, 32) for r0 in range(0, 256, 32)] + [rest]


def _store_wm(dst, wa, wb):
    RW = 48

    def blk(q, r0):
        w = [(wa, wb)[q % 2](k * QD + r0, k * QD + r0 + RW).astype(F32)
             for k in (2 * (q // 2), 2 * (q // 2) + 1)]
        return [w[r // 2][:, (r % 2) * L:(r % 2 + 1) * L] for r in range(4)]

    def job(o, r0):
        x, y, sg = _AC[o]
        oc = blk(x, r0)
        if sg:
            oc = [u + v if sg > 0 else u - v for u, v in zip(oc, blk(y, r0))]
        for i in range(7):
            dst[7 * o + i, r0:r0 + RW, :] = _combo(_AC, i, oc).astype(BF)
        return _token(jnp.maximum(_combo(_AC, 1, oc), _combo(_AC, 4, oc)))

    return [functools.partial(job, o, r0) for o in range(7) for r0 in range(0, QD, RW)]


def _store_nat(dst, t, v0, v1):
    rows = _Rows(pl.ds(pl.multiple_of(t * (L // 2), L // 2), L // 2))
    n1, n2 = v0.T, v1.T
    c = _acombos(n1[:, 0:256], n1[:, 256:512], n2[:, 0:256], n2[:, 256:512])
    for i in range(7):
        dst[i, rows, 0:256] = c[i].astype(BF)
    r1, r2 = n1[:, 512:D], n2[:, 512:D]
    dst[0, rows, 256:320] = r1.astype(BF)
    dst[1, rows, 256:320] = r2.astype(BF)
    dst[2, rows, 256:320] = r1.astype(BF)
    dst[5, rows, 256:320] = (r2 - r1).astype(BF)


def _nat_jobs(dst, t, src):
    rows = _Rows(pl.ds(pl.multiple_of(t * (L // 2), L // 2), L // 2))

    def main(c0):
        c = _acombos(*[src(h, k + c0, k + c0 + L).T for h in range(2) for k in (0, 256)])
        for i in range(7):
            dst[i, rows, c0:c0 + L] = c[i].astype(BF)
        return c[0][L - 8:L] + c[5][L - 8:L] + c[6][L - 8:L]

    def rest():
        r1, r2 = src(0, 512, D).T, src(1, 512, D).T
        dst[0, rows, 256:320] = r1.astype(BF)
        dst[1, rows, 256:320] = r2.astype(BF)
        dst[2, rows, 256:320] = r1.astype(BF)
        dst[5, rows, 256:320] = (r2 - r1).astype(BF)

    return [functools.partial(main, 0), functools.partial(main, L), rest]


def _tc_jobs(dst, src, t, plain=False):
    return [functools.partial(_store_tc, dst, src, t // 2, t % 2, r0, plain)
            for r0 in range(0, 80, RB)]


def _store_tc(dst, src, s, half, r0, plain):
    if isinstance(half, int):
        rd = lambda k: slice(half * 64 + k * QD + r0, half * 64 + k * QD + r0 + RB)
        wr = rd(0)
    else:
        rd = lambda k: pl.ds(pl.multiple_of(half * 64 + k * QD + r0, RB), RB)
        wr = _Rows(pl.ds(pl.multiple_of(half * 32 + r0 // 2, RB // 2), RB // 2))
    blk = [[src[2 * s + r // 2, q // 2, rd(2 * (q % 2) + r % 2), :].astype(F32)
            for r in range(4)] for q in range(4)]

    last = []

    def emit(o, i, v):
        dst[s, 7 * o + i % 7, wr, :] = v.astype(BF)
        last.append(v)

    _combos2(_BC, blk, emit, *(((), range(4)) if plain else ()))
    if plain:
        tk = functools.reduce(jnp.maximum, last[-8:])
        return jnp.maximum(tk[0:8], tk[8:16])


def _tc_half(dst, src, t, plain=False):
    for r0 in range(0, 80, RB):
        _store_tc(dst, src, t // 2, t % 2, r0, plain)


_LAST = []
_TOKS = []


def _run(jobs):
    for j in jobs:
        tok = j()
        if tok is not None:
            _TOKS.append(tok)


def _tie(v):
    top = v[0:8, 0:L]
    _LAST[:] = [top]
    if not _TOKS:
        return v
    for tok in _TOKS:
        top = jnp.minimum(top, jnp.maximum(top, tok))
    _TOKS.clear()
    if v.shape[1] > L:
        top = _cat([top, v[0:8, L:]])
    return _cat([top, v[8:]], 0)


def _kernel(x_hbm, g_hbm, wqkv_hbm, wo_hbm, w1_hbm, b1_hbm, w2_hbm, b2_hbm,
            out_hbm, dx_hbm, dwqkv_hbm, dwo_hbm, dw1_hbm, db1_hbm, dw2_hbm, db2_hbm, pre_hbm, hc_hbm,
            gin, wqs, wcat, wo, wbuf,
            X, OA, DA, N0, N1, Y0, Y1, QK0, QK1, STAT,
            YA, GA, TA, TB, HD2, WB, WA, PST,
            wqkT, wv, wvT, bmask, b2c,
            G0, G1, KV, KVT0, KVT1, M0, M1, MT, ZM, ZC0, ZC1,
            ACC, ZACC, DG, DKV, DKVT, DZC,
            DWS, DB1, DB2, DWQK, DWVT, DWO, b1, db1s, db2s, ZR, PS,
            sem_in, sem_x, sem_out, sem_o, sem_w, sem_wo, sem_wi, sem_ps, sem_pl, sem_h):
    (wcat, N0, N1, YA, GA, TA, TB,
     wqkT, wvT, bmask, G0, G1, KV, KVT0, KVT1, M0, M1, MT, ZM, DG, DKV, DKVT) = map(
         _Pk, (wcat, N0, N1, YA, GA, TA, TB,
               wqkT, wvT, bmask, G0, G1, KV, KVT0, KVT1, M0, M1, MT, ZM, DG, DKV, DKVT))
    Ns, Ys, QKs = (N0, N1), (Y0, Y1), (QK0, QK1)
    Gs, KVTs, Ms, ZCs = (G0, G1), (KVT0, KVT1), (M0, M1), (ZC0, ZC1)
    HC, DC = HD2.at[0], HD2.at[1]
    xin = Y1
    P = functools.partial
    _TOKS.clear()
    MB = (slice(0, HD), slice(HD, D))
    LN = (slice(0, L), slice(L, 2 * L))
    QR = [slice(k * QD, (k + 1) * QD) for k in range(4)]

    def tok(t, h):
        return pl.ds(pl.multiple_of(h * HS + t * L, L), L)

    def two(ref, t, r0, r1):
        return _cat([ref[t, 0, r0:r1, :], ref[t, 1, r0:r1, :]])

    def recomb(acc, nacc, t, h):
        if h == 0:
            m3 = acc[t, 3]
            top = acc[t, 0] + m3 - acc[t, 4]
            if nacc == 7:
                top = top + acc[t, 6]
            return _cat([top, acc[t, 1] + m3], 0)
        m2 = acc[t, 2]
        bot = acc[t, 0] - acc[t, 1] + m2
        if nacc == 7:
            bot = bot + acc[t, 5]
        return _cat([m2 + acc[t, 4], bot], 0)

    def lag(t, n=2):
        return max(t - n, 0) if isinstance(t, int) else jnp.maximum(t - n, 0)

    def zero_at(ref, t, i):
        z = jnp.minimum(0.0, jnp.maximum(0.0, _LAST[0]))
        ref[t, i] = _cat([z] * (HD // 8), 0)

    def zero(ref, *lead):
        ref[lead if lead else Ellipsis] = jnp.zeros(ref.shape[len(lead):], ref.dtype)

    cp = pltpu.make_async_copy

    def x_copy(t, h):
        return cp(x_hbm.at[:, tok(t, h)], xin.at[t, h], sem_x.at[2 * t + h])

    def g_copy(t, h):
        return cp(g_hbm.at[:, tok(t, h)], gin.at[t, h], sem_o.at[2 * t + h])

    def out_copy(t, h):
        return [cp(DC.at[4 * t + 2 * h + mb, pl.ds(0, HD)], out_hbm.at[MB[mb], tok(t, h)],
                   sem_o.at[4 * t + 2 * h + mb]) for mb in range(2)]

    def dx_copy(t, h):
        return cp(gin.at[t, h], dx_hbm.at[:, tok(t, h)], sem_x.at[2 * t + h])

    def fcols(j):
        return pl.ds(pl.multiple_of(j * T1, T1), T1)

    def ccols(j):
        return pl.ds(pl.multiple_of(j * 2 * T1, 2 * T1), 2 * T1)

    def w_in_copies(g):
        return [cp(w.at[:, ccols(g % NC)], wbuf.at[g % 2, k, :, pl.ds(0, 2 * T1)],
                   sem_w.at[2 * (g % 2) + k]) for k, w in enumerate((w1_hbm, w2_hbm))]

    def dw_copies(j, out):
        cs = []
        for k, w in enumerate((dw1_hbm, dw2_hbm)):
            hbm, buf = w.at[:, ccols(j)], DWS.at[j % 3, k, :, pl.ds(0, 2 * T1)]
            ix = 2 * (j % 3) + k
            cs.append(cp(buf, hbm, sem_wo.at[ix]) if out else cp(hbm, buf, sem_wi.at[ix]))
        return cs

    WQ = 384
    wq_copies = [cp(wqkv_hbm.at[:, pl.ds(k * WQ, WQ)], wqs.at[:, pl.ds(k * WQ, WQ)], sem_in.at[k])
                 for k in range(3)]
    in_copies = [cp(wqkv_hbm.at[:, pl.ds(2 * D, D)], wv, sem_in.at[3]),
                 cp(wo_hbm, wo, sem_in.at[4]),
                 cp(b2_hbm, db2s, sem_in.at[5]),
                 cp(b1_hbm, db1s, sem_in.at[6])]
    x_copy(0, 0).start()
    x_copy(0, 1).start()
    for c in wq_copies:
        c.start()
    x_copy(1, 0).start()
    x_copy(1, 1).start()

    for j, (r0, r1, t0, t1) in enumerate(PIECES):
        ri = (lax.broadcasted_iota(jnp.int32, (160, 128), 0) + r0).astype(F32)
        ci = (lax.broadcasted_iota(jnp.int32, (160, 128), 1) + t0).astype(F32)
        same = jnp.floor((ri + 0.5) * (1.0 / DH)) == jnp.floor((ci + 0.5) * (1.0 / DH))
        bmask[j] = jnp.where(same, 1.0, 0.0).astype(BF)
    for r in (ACC, ZACC, DWQK, DWVT, DWO, DB1, DB2):
        zero(r)

    def rrows(acc, nacc, t, h, k):
        A = lambda i: acc[t, i, (k % 2) * QD:(k % 2 + 1) * QD, :]
        if h == 0:
            if k >= 2:
                return A(1) + A(3)
            v = A(0) + A(3) - A(4)
            return v + A(6) if nacc == 7 else v
        if k < 2:
            return A(2) + A(4)
        v = A(0) - A(1) + A(2)
        return v + A(5) if nacc == 7 else v

    def fold(v):
        return jnp.broadcast_to(jnp.sum(v, axis=0, keepdims=True), (8, L))

    def psum(t, h, i, c):
        p = [PS[t, h, i, 8 * k + c:8 * k + c + 1, :] for k in range(4)]
        return (p[0] + p[1]) + (p[2] + p[3])

    def mix(x, y):
        return [j for i, m in enumerate(x)
                for j in [m] + y[i * len(y) // len(x):(i + 1) * len(y) // len(x)]]

    def put_stats(t, h, k, x):
        m = fold(x) * (1.0 / QD)
        c = x - m[0:1]
        PS[t, h, 0, 8 * k:8 * k + 8, :] = m
        PS[t, h, 1, 8 * k:8 * k + 8, :] = c = fold(c * c)
        return c

    def get_stats(t, h, c):
        m = psum(t, h, 0, c) * 0.25
        e = [PS[t, h, 0, 8 * k + c:8 * k + c + 1, :] - m for k in range(4)]
        return m, psum(t, h, 1, c) * (1.0 / D) + ((e[0] * e[0] + e[1] * e[1])
                                                  + (e[2] * e[2] + e[3] * e[3])) * 0.25

    def c_sum(l, t, h, k):
        if l == 0:
            x = xin[t, h, QR[k], :].astype(F32)
        else:
            x = X[t, h, QR[k], :] + rrows(OA, 5, t, h, k) + b2c[QR[k], :]
        X[t, h, QR[k], :] = x
        return put_stats(t, h, k, x)

    def c_app(l, t, h, k):
        m, v = get_stats(t, h, k)
        r = lax.rsqrt(v + EPS)
        n = (X[t, h, QR[k], :] - m) * r
        Ns[l][t, h, QR[k], :] = n.astype(BF)
        if k == 0:
            STAT[t, 8 * l:8 * l + 8, LN[h]] = jnp.broadcast_to(r, (8, L))
        return n[QD - 8:QD]

    def hk(f, l, t):
        return [P(f, l, t, h, k) for h in range(2) for k in range(4)]

    def c_zero(l, t):
        return ([P(zero_at, OA, t, i) for i in range(5)]
                + [P(zero_at, DA, t, i) for i in range(7 - 7 * l)])

    def c_qk(l, t, k):
        qk = _tie(_dot(wqkT[k * QD:(k + 1) * QD, :], two(Ns[l], t, 0, D)))
        ph = jnp.where(qk > 0, qk + 1.0, jnp.exp(jnp.minimum(qk, 0.0))) + PEPS
        r0 = k * QD if k < 4 else 2 * D + (k - 4) * QD
        for h in range(2):
            QKs[l][t, h, r0:r0 + QD, :] = ph[:, LN[h]].astype(BF)
        if k >= 4:
            ZACC[QR[k - 4], :] += ph[:, LN[0]] + ph[:, LN[1]]

    def c_g(l, t, k, n):
        c0, c1 = ((0, 256), (256, D))[n]
        r0 = 2 * D + k * QD
        ACC[QR[k], c0:c1] += _tie(_dot(two(QKs[l], t, r0, r0 + QD), two(Ns[l], t, c0, c1), NT))

    def g_db(t):
        DB2[...] += gin[t, 0].astype(F32) + gin[t, 1].astype(F32)

    def c_step(l, t, ahead, extra=()):
        v = (hk(c_sum, l, t + 2) if ahead >= 2 else []) + (hk(c_app, l, t + 1) if ahead else [])
        w = c_zero(l, t)
        st = isinstance(t, int)
        if l == 1:
            w = mix(w, _nat_jobs(GA, t, lambda h, r0, r1: gin[t, h, r0:r1, :].astype(F32))
                    + [P(g_db, t)])
        elif not (st and t == 0):
            w = mix(w, _tc_jobs(TA, gin, t - 1) + (_tc_jobs(TA, gin, t) if ahead == 0 else []))
        w = mix(w, list(extra)) if extra else w
        ms = [P(c_qk, l, t, 4 + k) for k in range(4)]
        for k in range(4):
            ms += [P(c_g, l, t, k, 0), P(c_qk, l, t, k), P(c_g, l, t, k, 1)]
        _run(mix(ms[:-1], mix(v, w) if v else w) + ms[-1:])
        if l == 1 or ahead == 0:
            return
        if st and t == 0:
            _run([x_copy(3, 0).wait, x_copy(3, 1).wait, g_copy(0, 0).wait, g_copy(0, 1).wait])
        g_copy(t + 1, 0).wait()
        g_copy(t + 1, 1).wait()
        if not st:
            @pl.when(t + 3 < NS)
            def _():
                x_copy(t + 3, 0).wait()
                x_copy(t + 3, 1).wait()

            @pl.when(t == 2)
            def _():
                _run([c.start for c in in_copies + w_in_copies(0)])

            @pl.when(t == 4)
            def _():
                _run([c.start for c in w_in_copies(1)])

    def loop(n, step):
        def body(t, carry):
            step(t)
            _TOKS.clear()
            return carry
        _TOKS.clear()
        lax.fori_loop(0, n, body, 0)

    def phase_c(l):
        if l == 0:
            c_step(l, 0, 2)
            loop(NS - 3, lambda t: c_step(l, t + 1, 2))
            _run([c.wait for c in w_in_copies(0)])
        else:
            loop(NS - 2, lambda t: c_step(l, t, 2))
        c_step(l, NS - 2, 1, (bwd_pro() if l else fwd_pro())[0:PRO[l][2]])

    def fin_fwd(l, jobs):
        def tie(v, n):
            if v.shape[1] < L:
                return v
            _run(jobs[0:n])
            del jobs[0:n]
            return _tie(v)

        Gs[l][...] = ACC[...].astype(BF)
        za = ZACC[...]
        ZR[:, 0:D] = jnp.sum(za.T, axis=0, keepdims=True)
        ZCs[l][...] = jnp.broadcast_to(jnp.sum(za, axis=1, keepdims=True), (D, 128))
        zero(ACC)
        zero(ZACC)
        for j, (r0, r1, t0, t1) in enumerate(PIECES):
            mk = bmask[j, 0:r1 - r0, 0:t1 - t0].astype(F32)
            KV[j, 0:r1 - r0, 0:t1 - t0] = (
                tie(_dot(Gs[l][r0:r1, :], wv[:, t0:t1]), PRO[l][1]) * mk).astype(BF)
            ZM[j, 0:r1 - r0, 0:t1 - t0] = (mk * ZR[:, t0:t1]).astype(BF)
        m = _bd_left(KV, lambda t0, t1: wo[t0:t1, :])
        Ms[l][...] = m.astype(BF)
        MT[...] = m.T.astype(BF)
        _run(jobs)

    def kvt(l):
        for j, (r0, r1, t0, t1) in enumerate(PIECES):
            mk = bmask[j, 0:r1 - r0, 0:t1 - t0].astype(F32)
            KVTs[l][j, 0:r1 - r0, 0:t1 - t0] = (
                _dot(wvT[r0:r1, :], Gs[l][t0:t1, :], NT) * mk).astype(BF)

    def a_s1(l, t, h):
        den = _bd_left(ZM, lambda t0, t1: QKs[l][t, h, t0:t1, :]) + PEPS
        rden = pl.reciprocal(den, approx=True)
        rden = rden * (2.0 - den * rden)
        pq = QKs[l][t, h, 0:D, :].astype(F32)
        QKs[l][t, h, D:2 * D, :] = (pq * rden).astype(BF)
        QKs[l][t, h, 0:D, :] = (rden * jnp.minimum(pq - PEPS, 1.0)).astype(BF)

    def a_xm(l, t, mb):
        v = _dot(MT[MB[mb], :], two(QKs[l], t, D, 2 * D))
        for h in range(2):
            X[t, h, MB[mb], :] += v[:, LN[h]]

    def a_tail(l, t):
        y = [None, None]

        def ln(h):
            x = X[t, h]
            c = x - _colmean(x)
            s = lax.rsqrt((1.0 + EPS) * _colmean(c * c) + EPS * EPS)
            y[h] = c * s
            Ys[l][t, h] = y[h].astype(BF)
            STAT[t, 16 + 8 * l:24 + 8 * l, LN[h]] = jnp.broadcast_to(s, (8, L))

        def tb():
            if l == 1:
                _tc_half(TB, Y1, lag(t))

        return [P(ln, 0), P(ln, 1), lambda: _store_nat(YA, t, y[0], y[1]), tb]

    def a_step(l, t, xm, s1):
        nop = lambda: None
        tl = a_tail(l, t)
        xj = [P(a_xm, l, t + 1, 0), P(a_xm, l, t + 1, 1)] if xm else [nop, nop]
        sj = [P(a_s1, l, t + 2, 0), P(a_s1, l, t + 2, 1)] if s1 else [nop, nop]
        _run([xj[0], tl[0], tl[1], xj[1], tl[2], sj[0], tl[3], sj[1]])

    def a_pro(l):
        _run([P(a_s1, l, 0, 0), P(a_s1, l, 0, 1), P(a_s1, l, 1, 0), P(a_xm, l, 0, 0),
              P(a_s1, l, 1, 1), P(a_xm, l, 0, 1)])

    def phase_a(l):
        loop(NS - 2, lambda t: a_step(l, t, True, True))
        a_step(l, NS - 2, True, False)
        a_step(l, NS - 1, False, False)
        if l == 1:
            kvt(1)
            _tc_half(TB, Y1, NS - 2)
            _tc_half(TB, Y1, NS - 1)

    def pre_store_copy(j):
        return cp(PST.at[j % 2], pre_hbm.at[j], sem_ps.at[j])

    def pre_load_copy(j):
        return cp(pre_hbm.at[j], PST.at[j % 2], sem_pl.at[j])

    def hc_store_copy(j):
        return cp(HD2.at[j % 2, pl.ds(0, 28), pl.ds(0, NQ * L)], hc_hbm.at[j], sem_h.at[j % 2])

    def hc_load_copy(j, k):
        tiles = (pl.ds(0, 16), pl.ds(16, 12))[k]
        return cp(hc_hbm.at[j, tiles], HC.at[tiles, pl.ds(0, NQ * L)], sem_h.at[k])

    def wsrc(g, k):
        return [(lambda r0, r1, a=a: wbuf[g % 2, k, r0:r1, a * T1:(a + 1) * T1]) for a in range(2)]

    def store_wk(slot, g, k):
        return _store_wk(_Pk(WB.at[slot]), *wsrc(g, k))

    def store_wm(slot, g, k):
        return _store_wm(_Pk(WA.at[slot]), *wsrc(g, k))

    full = dict(YA=YA, GA=GA, HC=HC, DC=DC, OA=OA, DA=DA, X=X)

    def views(k):
        rows = pl.ds(pl.multiple_of(k * 2 * L, 2 * L), 2 * L)
        ts = pl.ds(4 * k, 4)
        return dict(YA=_Pk(YA.ref.at[:, rows]), GA=_Pk(GA.ref.at[:, rows]), HC=HC.at[:, rows],
                    DC=DC.at[:, rows], OA=OA.at[ts], DA=DA.at[ts], X=X.at[ts])

    def first_stage(As, s, r0, b):
        rr = [2 * L * s + p * L + r0 for p in range(2)]
        m = [[None] * 7 for _ in As]
        for grp in ((2, 4), (1, 3), (0, 6), (5,)):
            for k, A in enumerate(As):
                for i in grp:
                    if A is not None:
                        m[k][i] = _dot(_cat([A[i, r:r + R1, 0:KW[i]] for r in rr], 0),
                                       _Pk(WB.at[k])[i, 0:KW[i], LN[b]])
        return m

    def quad(m, r, p):
        r = p * R1 + r
        return _recomb([x[r:r + RB] for x in m])

    def store_hc(dst, v, r, plain=()):
        sums = []

        def emit(o, i, c):
            dst[_hix(o, i), r:r + RB, :] = c.astype(BF)
            if o >= 5 and i in (5, 6):
                sums.append(c)

        _combos2(_BC, [[v[k][2 * (q % 2) + q // 2] for k in range(4)] for q in range(4)], emit,
                 plain=plain)
        return sums

    def second(V, slot, out, o, s):
        W = _Pk(WA.at[slot])
        src = V['HC' if out else 'DC']
        c = [_dot(W[7 * o + i], src[_hix(o, i), s * L:(s + 1) * L, :], NT) for i in range(7)]
        c = _recomb(c[0:6] + [_tie(c[6])])
        for q in range(4):
            t, r = 2 * s + q % 2, (q // 2) * QD
            if not out:
                V['DA'][t, o, r:r + QD, :] += c[q]
            elif o == 6:
                V['X'][t, 0, r:r + QD, :] += c[q]
            elif o == 5:
                V['X'][t, 1, HD + r:HD + r + QD, :] += c[q]
            else:
                V['OA'][t, o, r:r + QD, :] += c[q]

    def pst_ix(j, q, k, s, r):
        r = (q // 2) * HS + (2 * s + k % 2) * L + r
        return (j % 2, 2 * (q % 2) + k // 2, slice(r, r + RB), slice(None))

    def bias_of(j):
        v = [b1[:, fcols(2 * j + a)] for a in range(2)]
        return [[v[a][:, LN[b]] for b in range(2)] for a in range(2)]

    def pop(jobs, n):
        for _ in range(n):
            if jobs:
                _run([jobs.pop(0)])

    def fwd_pro():
        return store_wk(1, 0, 0) + store_wm(1, 0, 1)

    def mlp_fwd():
        def step(j):
            for c in w_in_copies(j + 2):
                c.start()
            for c in w_in_copies(j + 1):
                c.wait()

            @pl.when(j >= 1)
            def _():
                pre_store_copy(j - 1).start()
                hc_store_copy(j - 1).start()

            @pl.when(j >= 2)
            def _():
                pre_store_copy(j - 2).wait()
                hc_store_copy(j - 2).wait()

            V = dict(full, HC=HD2.at[j % 2])
            bias = bias_of(j)
            jobs = []
            for s in range(NQ):
                for r0 in range(0, L, R1):
                    hh = [[] for _ in range(0, R1, RB)]
                    for b in range(2):
                        Pm = first_stage((None, YA), s, r0, b)[1]
                        pop(jobs, 1 if r0 + b else 0)
                        for r in range(0, R1, RB):
                            for p in range(2):
                                pre = [v + bias[q % 2][b] for q, v in enumerate(quad(Pm, r, p))]
                                for q in range(4):
                                    PST[pst_ix(j, q, 2 * b + p, s, r0 + r)] = pre[q].astype(BF)
                                hh[r // RB].append([_gelu(v, False)[0] for v in pre])
                            if b == 1:
                                store_hc(V['HC'], hh[r // RB], s * L + r0 + r, (1, 2))
                if 1 <= s < NQ - 1:
                    jobs += [P(second, V, 1, True, o, s - 1) for o in range(7)]
            wk, wm = store_wk(1, j + 1, 0), store_wm(1, j + 1, 1)
            for o in range(7):
                second(V, 1, True, o, NQ - 2)
                pop(wk, 2)
                pop(wm, 1 if o else 0)
                second(V, 1, True, o, NQ - 1)
                pop(wm, 2 if o < 6 else 3)

        loop(NC, step)
        pre_store_copy(NC - 1).start()
        hc_store_copy(NC - 1).start()

    def bwd_pro():
        return store_wk(0, NC, 1) + store_wm(0, NC, 0)

    def mlp_bwd(l):
        g0 = (2 - l) * NC

        def blocks(j, V, ns, jobs, fill=()):
            if l == 1:
                bias = bias_of(j)
            acc = [jnp.zeros((8, L), F32)] * 4
            for s in range(ns):
                for r0 in range(0, L, R1):
                    hh = [[] for _ in range(0, R1, RB)]
                    dp = [[] for _ in range(0, R1, RB)]
                    for b in range(2):
                        Q, Pm = first_stage((V['GA'], V['YA'] if l else None), s, r0, b)
                        pop(jobs, (l + 1) if r0 + b else 0)
                        pop(fill, FILL[s] if fill else 0)
                        for r in range(0, R1, RB):
                            for p in range(2):
                                if l == 1:
                                    pre = [v + bias[q % 2][b]
                                           for q, v in enumerate(quad(Pm, r, p))]
                                else:
                                    pre = [PST[pst_ix(j, q, 2 * b + p, s, r0 + r)].astype(F32)
                                           for q in range(4)]
                                hg = [_gelu(v, True) for v in pre]
                                hh[r // RB].append([v[0] for v in hg])
                                dp[r // RB].append([d * v[1] for d, v in zip(quad(Q, r, p), hg)])
                            if b == 1:
                                if l == 1:
                                    store_hc(V['HC'], hh[r // RB], s * L + r0 + r)
                                sm = store_hc(V['DC'], dp[r // RB], s * L + r0 + r)
                                acc = [acc[k] + jnp.sum(sm[k].reshape(RB // 8, 8, L), axis=0)
                                       for k in range(4)]
                for o in range(7):
                    if l == 1:
                        jobs.append(P(second, V, 1, True, o, s))
                    jobs.append(P(second, V, 0, False, o, s))
            DB1[:, ccols(j)] += _cat(acc)

        def dw(j, k, T, src, plain=False):
            lhs = lambda e, r0, r1: [T[s, e, r0:r1, :] for s in range(NQ)]
            ni = 4 if plain else 7

            def prod(m, r0, r1, o, i):
                if plain:
                    a = lhs(7 * o + i % 2, r0, r1) + lhs(7 * o + 2 + i % 2, r0, r1)
                    b = _cat([src[_hix(A2B[o], 7 + 2 * (i // 2) + p), 0:NQ * L, :]
                              for p in range(2)], 0)
                else:
                    a = lhs(7 * o + i, r0, r1)
                    b = src[_hix(A2B[o], A2B[i]), 0:NQ * L, :]
                if l == 1:
                    _TOKS.clear()
                m[o].append(_tie(_dot(_cat(a), b)))
                if i == 6:
                    m[o] = _recomb(m[o])
                if o != (1 if plain else 6) or i < ni - 1:
                    return
                for qi in range(4):
                    c = _recomb([m[o][qi] for o in range(7)])
                    for q in range(4):
                        rr = (q % 2) * HD + (qi % 2) * QD
                        cc = (q // 2) * T1 + (qi // 2) * L
                        ix = (j % 3, k, slice(rr + r0, rr + r1), slice(cc, cc + L))
                        v = c[q]
                        if l == 0:
                            v = v + DWS[ix].astype(F32)
                        DWS[ix] = v.astype(BF)

            rs = [([[] for _ in range(7)], r0, r1) for r0, r1 in ((0, 80), (80, QD))]
            if plain:
                return [P(prod, *r, o, i) for o in (0, 2, 6, 5, 3, 4, 1) for r in rs
                        for i in range(ni)]
            return [P(prod, *r, o, i) for r in rs for o in range(7) for i in range(ni)]

        def with_extra(jobs, extra, den):
            return [x for n, p in enumerate(jobs)
                    for x in (extra[n // den:n // den + 1] if n % den == den - 1 else []) + [p]]

        def step(j):
            g = g0 + j
            jobs = []

            @pl.when(j >= 1)
            def _():
                for c in dw_copies(j - 1, True):
                    c.start()

            @pl.when(j >= 2)
            def _():
                for c in dw_copies(j - 2, True):
                    c.wait()

            if l == 0:
                @pl.when(j + 1 < NC)
                def _():
                    pre_load_copy(j + 1).start()
                    for c in dw_copies(j + 1, False):
                        c.start()
                    for c in w_in_copies(g + 1):
                        c.wait()

                @pl.when(j + 2 < NC)
                def _():
                    for c in w_in_copies(g + 2):
                        c.start()

                for c in dw_copies(j, False):
                    c.wait()
                hc_load_copy(j, 1).wait()
                hc_load_copy(j, 0).wait()
                pre_load_copy(j).wait()

                def hc_next(k):
                    @pl.when(j + 1 < NC)
                    def _():
                        hc_load_copy(j + 1, k).start()

                fill = dw(j, 1, TB, HC, True)
                fill = fill[0:32] + [P(hc_next, 0)] + fill[32:]
                blocks(j, full, NQ, jobs, fill)
                _run(fill[0:4] + mix(jobs, fill[4:]))
                hc_next(1)
                _run(with_extra(dw(j, 0, TA, DC),
                                store_wk(0, g + 1, 1) + store_wm(0, g + 1, 0), 3))
            else:
                for c in w_in_copies(g + 2):
                    c.start()
                for c in w_in_copies(g + 1):
                    c.wait()

                def half(k):
                    blocks(j, views(k), 2, jobs)
                    _run(jobs)
                    jobs.clear()

                loop(NQ // 2, half)
                _run(with_extra(dw(j, 1, TA, HC), store_wk(0, g + 1, 1) + store_wm(0, g + 1, 0), 3))
                _run(with_extra(dw(j, 0, TB, DC), store_wk(1, g + 1, 0) + store_wm(1, g + 1, 1), 3))

        loop(NC, step)
        for c in dw_copies(NC - 1, True):
            c.start()

    def dw_drain():
        for j in (NC - 2, NC - 1):
            for c in dw_copies(j, True):
                c.wait()

    def e_sum(l, t, h, k):
        dy = rrows(DA, 7, t, h, k)
        PS[t, h, 0, 8 * k:8 * k + 8, :] = fold(dy)
        PS[t, h, 1, 8 * k:8 * k + 8, :] = tk = fold(dy * Ys[l][t, h, QR[k], :].astype(F32))
        if l == 1:
            out = X[t, h, QR[k], :] + rrows(OA, 5, t, h, k) + b2c[QR[k], :]
            DC[4 * t + 2 * h + k // 2, QR[k % 2], :] = out.astype(BF)
            tk = tk + jnp.max(out.reshape(QD // 8, 8, L), axis=0)
        return tk

    def e_app(l, t, h, k):
        dy = rrows(DA, 7, t, h, k)
        s = STAT[t, 16 + 8 * l + k:17 + 8 * l + k, LN[h]]
        m1, m2 = psum(t, h, 0, k) * (1.0 / D), psum(t, h, 1, k) * ((1.0 + EPS) / D)
        dx = s * (dy - m1 - Ys[l][t, h, QR[k], :].astype(F32) * m2)
        dx = dx + (gin[t, h, QR[k], :].astype(F32) if l == 1 else X[t, h, QR[k], :])
        X[t, h, QR[k], :] = dx
        Ys[l][t, h, QR[k], :] = dx.astype(BF)
        return dx[QD - 8:QD]

    def e_apps(l, t):
        return hk(e_app, l, t)

    def e_sums(l, t):
        return hk(e_sum, l, t)

    def e_step(l, t, ahead):
        dp = [None] * 5
        ps = [None] * 5

        def j_dp(j, h):
            t0, t1 = PIECES[j][2:]
            v = _tie(_dot(Ms[l][t0:t1, :], Ys[l][t, h]))
            dp[j] = _cat([dp[j], v]) if h else v

        def j_acc(k, n):
            c0, c1 = ((0, 256), (256, D))[n]
            ACC[QR[k], c0:c1] += _tie(_dot(two(QKs[l], t, D + k * QD, D + (k + 1) * QD),
                                           two(Ys[l], t, c0, c1), NT))

        def j_dq(j):
            r0, r1, t0, t1 = PIECES[j]
            tt = (dp[j] * two(QKs[l], t, D + t0, D + t1).astype(F32)).astype(BF)
            ps[j] = _dot(bmask[j, 0:r1 - r0, 0:t1 - t0], tt)
            hi = r1 if j == 4 else PIECES[j + 1][0]
            d, hs = dp[j][0:hi - t0], ps[j][0:hi - r0]
            if j:
                d = _cat([dp[j - 1][L - 16:L], d], 0)
                hs = _cat([hs[0:32] + ps[j - 1][r0 - PIECES[j - 1][0]:], hs[32:]], 0)
            z = None
            for h in range(2):
                cq = QKs[l][t, h, r0:hi, :].astype(F32)
                QKs[l][t, h, r0:hi, :] = (
                    cq * (d[:, LN[h]] - ZCs[l][r0:hi, :] * hs[:, LN[h]])).astype(BF)
                w = QKs[l][t, h, D + r0:D + hi, :].astype(F32) * hs[:, LN[h]]
                z = w if z is None else z + w
            ZACC[r0:hi, :] += z

        v = (e_sums(l, t + 2) if ahead >= 2 else []) + (e_apps(l, t + 1) if ahead >= 1 else [])
        for m in 'p0 p1 q0 a0 p2 q1 a1 p3 q2 p4 a2 q3 q4 a3'.split():
            if m[0] == 'q':
                j_dq(int(m[1]))
                continue
            for h in range(2):
                (j_dp if m[0] == 'p' else j_acc)(int(m[1]), h)
                pop(v, 1)

    def e_pro(l):
        _run(e_sums(l, 0) + e_sums(l, 1) + e_apps(l, 0))

    def phase_e(l):
        loop(NS - 2, lambda t: e_step(l, t, 2))
        e_step(l, NS - 2, 1)

    def fin_bwd(l):
        DG[...] = ACC[...].astype(BF)
        DZC[...] = jnp.broadcast_to(-jnp.sum(ZACC[...], axis=1, keepdims=True), (D, 128))
        if l == 1:
            zero(ACC)
            zero(ZACC)
        for j, (r0, r1, t0, t1) in enumerate(PIECES):
            mk = bmask[j, 0:r1 - r0, 0:t1 - t0].astype(F32)
            DKV[j, 0:r1 - r0, 0:t1 - t0] = (_dot(DG[r0:r1, :], wo[t0:t1, :], NT) * mk).astype(BF)
        dg = _bd_left(DKV, lambda t0, t1: wvT[t0:t1, :])
        MT[...] = dg.astype(BF)
        wcat[:, 2 * D:3 * D] = dg.T.astype(BF)
        for j, (r0, r1, t0, t1) in enumerate(PIECES):
            mk = bmask[j, 0:r1 - r0, 0:t1 - t0].astype(F32)
            DKVT[j, 0:r1 - r0, 0:t1 - t0] = (_dot(wo[r0:r1, :], DG[t0:t1, :], NT) * mk).astype(BF)
        DWO[...] += _bd_left(KVTs[l], lambda t0, t1: DG[t0:t1, :])
        DWVT[...] += _bd_left(DKVT, lambda t0, t1: Gs[l][t0:t1, :])

    def f_dk(l, t, k):
        dpk = _tie(_dot(MT[QR[k], :], two(Ns[l], t, 0, D)))
        r0 = 2 * D + k * QD
        for h in range(2):
            pk = QKs[l][t, h, r0:r0 + QD, :].astype(F32)
            QKs[l][t, h, r0 - D:r0 - D + QD, :] = (
                (dpk[:, LN[h]] + DZC[QR[k], :]) * jnp.minimum(pk - PEPS, 1.0)).astype(BF)

    def f_w(l, t, k, n):
        c0, c1 = ((0, 512), (512, 2 * D))[n]
        DWQK[QR[k], c0:c1] += _tie(
            _dot(two(Ns[l], t, k * QD, (k + 1) * QD), two(QKs[l], t, c0, c1), NT))

    def f_s1(l, t):
        return ([P(f_dk, l, t, k) for k in range(4)]
                + [P(f_w, l, t, k, n) for n in range(2) for k in range(4)])

    def f_dn(l, t, k, h):
        d = _tie(_dot(wcat[QR[k], :], QKs[l][t, h]))
        OA[t, 2 * h + k // 2, QR[k % 2], :] = d
        PS[t, h, 0, 8 * k:8 * k + 8, :] = fold(d)
        PS[t, h, 1, 8 * k:8 * k + 8, :] = fold(d * Ns[l][t, h, QR[k], :].astype(F32))

    def f_app(l, t, k):
        rr, ro = slice(96 * k, 96 * k + 96), slice(96 * (k % 3), 96 * (k % 3) + 96)
        dx = []
        for h in range(2):
            m1, m2 = psum(t, h, 0, k) * (1.0 / D), psum(t, h, 1, k) * (1.0 / D)
            n = Ns[l][t, h, rr, :].astype(F32)
            dx.append(X[t, h, rr, :]
                      + STAT[t, 8 * l + k:8 * l + k + 1, LN[h]]
                      * (OA[t, 2 * h + k // 3, ro, :] - m1 - n * m2))
            if l == 1:
                X[t, h, rr, :] = dx[h]
            else:
                gin[t, h, rr, :] = dx[h].astype(BF)
        if l == 1:
            DB2[rr, :] += dx[0] + dx[1]
        return dx[0][88:96] + dx[1][88:96]

    def f_apps(l, t):
        return [P(f_app, l, t, k) for k in range(6)]

    def f_nat(t):
        return _nat_jobs(GA, t, lambda h, r0, r1: X[t, h, r0:r1, :])

    def f_step(l, tp, extra=()):
        t = tp + 1
        first, last = isinstance(t, int) and t == 0, isinstance(t, int) and t == NS - 1
        v0, v1 = list(extra), [] if first else f_apps(l, tp)
        if l == 1:
            v0 = _tc_jobs(TB, X, lag(t, 3), True) + f_nat(lag(t))
            if last:
                v0 += _tc_jobs(TB, X, NS - 3, True)
            v0 = mix(v0, [P(zero_at, DA, t, i) for i in range(7)])
            v1 = mix(_tc_jobs(TA, Y0, t), v1) + (f_nat(NS - 2) if last else [])
        ms = [P(f_dn, l, t, k, h) for k in range(4) for h in range(2)]
        if not last:
            s1 = f_s1(l, tp + 2)
            ms = [m for i in range(4) for m in (ms[2 * i], s1[i], ms[2 * i + 1], s1[4 + i])] + s1[8:]
        n = len(ms) * 2 // 5 if v0 else 0
        _run(mix(ms[:n], v0) + mix(ms[n:-1], v1) + ms[-1:])
        if last:
            if l == 0:
                _run([dx_copy(t - 1, h).start for h in range(2)])
            _run(f_apps(l, t))
            if l == 1:
                kvt(0)
                _run(f_nat(t) + _tc_jobs(TB, X, NS - 2, True) + _tc_jobs(TB, X, NS - 1, True))
            else:
                _run([dx_copy(t, h).start for h in range(2)])

    def phase_f(l):
        f_step(l, -1)
        loop(NS - 2, lambda t: f_step(l, t))
        if l == 0:
            loop(NS - 2, lambda t: [dx_copy(t, h).start() for h in range(2)])

    def u0():
        x_copy(0, 0).wait()
        x_copy(0, 1).wait()
        _run(hk(c_sum, 0, 0) + hk(c_app, 0, 0))
        eye = jnp.where(lax.broadcasted_iota(jnp.int32, (L, L), 0)
                        == lax.broadcasted_iota(jnp.int32, (L, L), 1), 1.0, 0.0).astype(BF)
        for k in range(3):
            wq_copies[k].wait()
            if k == 0:
                _run([x_copy(2, h).start for h in range(2)])
            if k == 2:
                for t in range(3, NS + 3):
                    _run([x_copy(t, h).start for h in range(2) if t < NS]
                         + [g_copy(t - 3, h).start for h in range(2)])
                _run([x_copy(u, h).wait for u in (1, 2) for h in range(2)])
                _run(hk(c_sum, 0, 1))
            for c in range(k * WQ, (k + 1) * WQ, L):
                wq = wqs[:, c:c + L]
                wqkT[c:c + L, :] = _dot(eye, wq, NT).astype(BF)
                wcat[:, c:c + L] = wq

    _scoped('u0', u0)
    _scoped('phase_c0', phase_c, 0)
    for c in in_copies:
        c.wait()

    def mid_fwd(l):
        if l == 0:
            wvT[...] = wv[...].astype(F32).T.astype(BF)
            b2c[...] = jnp.broadcast_to(db2s[...].astype(F32).reshape(1, D), (128, D)).T
            b1[...] = db1s[...].astype(F32).reshape(1, F)
        jobs = (bwd_pro() if l else fwd_pro())[PRO[l][2]:]
        c_step(l, NS - 1, 0, jobs[0:PRO[l][0]])
        fin_fwd(l, jobs[PRO[l][0]:])
        a_pro(l)

    _scoped('mid_fwd0', mid_fwd, 0)
    _scoped('phase_a0', phase_a, 0)
    _scoped('mlp_fwd', mlp_fwd)
    def u1():
        _run(hk(c_sum, 1, 0) + hk(c_sum, 1, 1) + hk(c_app, 1, 0))

    _scoped('u1', u1)
    _scoped('phase_c1', phase_c, 1)
    for j in (NC - 2, NC - 1):
        pre_store_copy(j).wait()
        hc_store_copy(j).wait()
    _scoped('mid_fwd1', mid_fwd, 1)
    _scoped('phase_a1', phase_a, 1)
    _scoped('mlp_bwd1', mlp_bwd, 1)

    small = [cp(db1s, db1_hbm, sem_out.at[0]),
             cp(db2s, db2_hbm, sem_out.at[1]),
             cp(wo, dwo_hbm, sem_out.at[2]),
             cp(wv, dwqkv_hbm.at[:, pl.ds(2 * D, D)], sem_out.at[3]),
             cp(wqs, dwqkv_hbm.at[:, pl.ds(0, 2 * D)], sem_out.at[4])]

    def mid_bwd(l):
        e_step(l, NS - 1, 0)
        fin_bwd(l)
        _run(f_s1(l, 0))
        if l == 0:
            wo[...] = DWO[...].astype(BF)
            wv[...] = DWVT[...].T.astype(BF)
            small[2].start()
            small[3].start()

    _scoped('u2', e_pro, 1)
    _scoped('phase_e1', phase_e, 1)
    outs = [c for t in range(NS) for h in range(2) for c in out_copy(t, h)]
    _run([c.start for c in outs])
    dw_drain()
    _scoped('mid_bwd1', mid_bwd, 1)
    pre_load_copy(0).start()
    hc_load_copy(0, 0).start()
    hc_load_copy(0, 1).start()
    for c in dw_copies(0, False):
        c.start()
    _scoped('phase_f1', phase_f, 1)
    _run([c.wait for c in outs])
    _scoped('u3', f_step, 1, NS - 2)
    _scoped('mlp_bwd0', mlp_bwd, 0)
    db1s[...] = jnp.sum(DB1[...], axis=0).astype(BF)
    db2s[...] = jnp.sum(DB2[...].T, axis=0).astype(BF)
    small[0].start()
    small[1].start()
    _scoped('u4', e_pro, 0)
    _scoped('phase_e0', phase_e, 0)
    _scoped('mid_bwd0', mid_bwd, 0)
    _scoped('phase_f0', phase_f, 0)

    def flush_dwqk():
        wqs[...] = DWQK[...].astype(BF)
        small[4].start()

    _scoped('u5', f_step, 0, NS - 2, [flush_dwqk])
    dw_drain()
    for c in small:
        c.wait()
    for t in range(NS):
        dx_copy(t, 0).wait()
        dx_copy(t, 1).wait()


@jax.jit
def pallas_interleave_layers__linear_attn_block__mixer_channel_mlp__prompt_kernel(
    A_x: jax.Array,
    A_wqkv: jax.Array,
    A_wo: jax.Array,
    B_x: jax.Array,
    B_w1: jax.Array,
    B_b1: jax.Array,
    B_w2: jax.Array,
    B_b2: jax.Array,
    grad_out: jax.Array,
):
    del B_x
    xT = jnp.swapaxes(A_x[0], 0, 1)
    gT = jnp.swapaxes(grad_out[0], 0, 1)
    V = pltpu.VMEM

    def P(*shape):
        return V(shape[:-2] + (shape[-2] // 2, shape[-1]), U32)

    PC = P(5, 160, 128)
    DD = P(D, D)
    COL = V((D, 128), F32)
    BLK = V((NS, 2, D, L), BF)
    scratch = [
        BLK, V((D, 2 * D), BF), P(D, 3 * D), V((D, D), BF), V((2, 2, D, 5 * L), BF),
        V((NS, 2, D, L), F32), V((NS, 5, HD, L), F32), V((NS, 7, HD, L), F32),
        P(NS, 2, D, L), P(NS, 2, D, L), BLK, BLK,
        V((NS, 2, 3 * D, L), BF), V((NS, 2, 3 * D, L), BF), V((NS, 32, 2 * L), F32),
        P(7, HS, 384), P(7, HS, 384), P(NQ, 49, QD, L), P(NQ, 49, QD, L),
        V((2, 63, NQ * L + 16, L), BF),
        P(2, 7, 320, T1), P(2, 49, QD, L), V((2, 4, S, L), BF),
        P(2 * D, D), V((D, D), BF), DD, PC, COL,
        DD, DD, PC, PC, PC, DD, DD, DD, PC, COL, COL,
        V((D, D), F32), COL, DD, PC, PC, COL,
        V((3, 2, D, 5 * L), BF), V((8, F), F32), COL,
        V((D, 2 * D), F32), V((D, D), F32), V((D, D), F32),
        V((1, F), F32), V((F,), BF), V((D,), BF), V((1, 896), F32),
        V((NS, 2, 2, 32, L), F32),
        pltpu.SemaphoreType.DMA((7,)), pltpu.SemaphoreType.DMA((2 * NS,)),
        pltpu.SemaphoreType.DMA((5,)), pltpu.SemaphoreType.DMA((4 * NS,)),
        pltpu.SemaphoreType.DMA((4,)),
        pltpu.SemaphoreType.DMA((6,)), pltpu.SemaphoreType.DMA((6,)),
        pltpu.SemaphoreType.DMA((NC,)), pltpu.SemaphoreType.DMA((NC,)),
        pltpu.SemaphoreType.DMA((2,)),
    ]
    sds = jax.ShapeDtypeStruct
    outT, dxT, dwqkv, dwo, dw1, db1, dw2T, db2, _, _ = pl.pallas_call(
        _kernel,
        in_specs=[pl.BlockSpec(memory_space=pl.ANY)] * 8,
        out_specs=[pl.BlockSpec(memory_space=pl.ANY)] * 10,
        out_shape=[sds((D, S), BF), sds((D, S), BF), sds((D, 3 * D), BF), sds((D, D), BF),
                   sds((D, F), BF), sds((F,), BF), sds((D, F), BF), sds((D,), BF),
                   sds((NC, 4, S, L), BF), sds((NC, 28, NQ * L, L), BF)],
        scratch_shapes=scratch,
        compiler_params=pltpu.CompilerParams(vmem_limit_bytes=128 * 2**20,
                                             disable_bounds_checks=True),
    )(xT, gT, A_wqkv, A_wo, B_w1, B_b1, B_w2.T, B_b2)
    return (jnp.swapaxes(outT, 0, 1)[None], jnp.swapaxes(dxT, 0, 1)[None], dwqkv, dwo, dw1,
            db1, dw2T.T, db2)
```
